```python
import os as _os
_os.environ.setdefault("JAX_PLATFORMS", "cpu")
import jax
import jax.numpy as jnp

def _softmax(x, axis=-1):
    return jax.nn.softmax(x, axis=axis)
def _gelu(x):
    return jax.nn.gelu(x, approximate=True)
def _silu(x):
    return jax.nn.silu(x)
def _sigmoid(x):
    return jax.nn.sigmoid(x)
def _layernorm(x, axis=-1, eps=1e-5):
    m = jnp.mean(x, axis=axis, keepdims=True)
    v = jnp.var(x, axis=axis, keepdims=True)
    return (x - m) / jnp.sqrt(v + eps)
def _scatter_add(tgt, idx, src, axis=0):
    return tgt.at[idx].add(src)
def _segment_sum(src, seg, n):
    return jax.ops.segment_sum(src, seg, n)
class _Rng:
    def __init__(self, key):
        self._k = key
    def _next(self):
        self._k, sub = jax.random.split(self._k)
        return sub
    def normal(self, shape):
        return jax.random.normal(self._next(), shape, dtype=jnp.bfloat16)
    def randint(self, lo, hi, shape):
        return jax.random.randint(self._next(), shape, lo, hi, dtype=jnp.int32)
    def uniform(self, shape, lo=0.0, hi=1.0):
        return jax.random.uniform(self._next(), shape, jnp.bfloat16, lo, hi)
    def permutation(self, n):
        return jax.random.permutation(self._next(), n)


kernel_name = 'parallel_sum__mha_block__dense_activation_mish__prompt'

def setup_inputs():
    _rng = _Rng(jax.random.key(int.from_bytes(__import__("os").urandom(4), "little")))
    _w = (lambda a: (lambda t: t.astype(jnp.bfloat16) if jnp.issubdtype(t.dtype, jnp.floating) else t)(jnp.asarray(a)))
    def _A_setup():
        B, S, D, H = 1, 2048, 512, 32
        return {
            "x": _w((lambda *s: _rng.normal(s) * 0.05)(B, S, D)),
            "wqkv": _w((lambda *s: _rng.normal(s) * 0.05)(D, 3 * D)),
            "wo": _w((lambda *s: _rng.normal(s) * 0.05)(D, D)),
        }
    _A_in = _A_setup()

    def _B_setup():
        B, S, D, F = 1, 2048, 512, 1792
        return {
            "x": _w((lambda *s: _rng.normal(s) * 0.05)(B, S, D)),
            "w1": _w((lambda *s: _rng.normal(s) * 1.6)(D, F) * (D ** -0.5)),
            "b1": _w((lambda *s: _rng.normal(s) * 0.05)(F)),
            "w2": _w((lambda *s: _rng.normal(s) * 0.05)(F, D) * (F ** -0.5)),
        }
    _B_in = _B_setup()

    return {
        "A_x": _A_in["x"],
        "A_wqkv": _A_in["wqkv"],
        "A_wo": _A_in["wo"],
        "B_x": _B_in["x"],
        "B_w1": _B_in["w1"],
        "B_b1": _B_in["b1"],
        "B_w2": _B_in["w2"],
    }

def reference(A_x, A_wqkv, A_wo, B_x, B_w1, B_b1, B_w2):
    def _A_ref(x, wqkv, wo):
        B, S, D = x.shape
        H = 32
        Dh = D // H
        qkv = (lambda x, *d: x.transpose(*d))((x @ wqkv).reshape(B, S, 3, H, Dh), 2, 0, 3, 1, 4)
        q, k, v = qkv[0], qkv[1], qkv[2]
        scores = jnp.einsum("bhqd,bhkd->bhqk", q, k) * (Dh ** -0.5)
        p = _softmax(scores, axis=-1)
        o = jnp.einsum("bhqk,bhkd->bhqd", p, v)
        return (lambda x, *d: x.transpose(*d))(o, 0, 2, 1, 3).reshape(B, S, D) @ wo

    def _B_ref(x, w1, b1, w2):
        h = jnp.einsum("bsd,df->bsf", x, w1) + b1
        sp = jnp.log1p(jnp.exp(-jnp.abs(h))) + jnp.where(h > 0, h, jnp.zeros_like(h))
        act = h * jnp.tanh(sp)
        return jnp.einsum("bsf,fd->bsd", act, w2)

    x = A_x
    xn = _layernorm(x, axis=-1)
    return x + _A_ref(xn, A_wqkv, A_wo) + _B_ref(xn, B_w1, B_b1, B_w2)
```

```python
import functools
import math

import jax
import jax.numpy as jnp
from jax import lax
import jax.experimental.pallas as pl
import jax.experimental.pallas.tpu as pltpu

_H = 32
_EPS = 1e-5
_LANES = 128

F32 = jnp.float32
BF16 = jnp.bfloat16
U32 = jnp.uint32


def _pack(a):
    return pltpu.bitcast(a, U32)


def _unpack(a):
    return pltpu.bitcast(a, BF16)


def _vreg_max(a):
    return jnp.max(a.reshape(a.shape[0] // 8, 8, a.shape[1]), axis=0)


def _vreg_sum(a):
    return jnp.sum(a.reshape(a.shape[0] // 8, 8, a.shape[1]), axis=0)


def _kernel(x_hbm, wqkv_hbm, wo_hbm, w1_hbm, b1_hbm, w2_hbm, out_hbm,
            x_v, wqkv_v, wo_v, w1_v, b1_v, w2_v, out_v,
            xn_s, qt_s, k_s, vt_s, qm_s, s_s, ot_s, l_s, sems, osems,
            *, S, D, F, TQ, CK, RB, UNROLL, FB, OB, FENCE, G, LAG):
    dh = D // _H
    hpg = _LANES // dh
    ng = D // _LANES
    nqb = S // TQ
    nch = S // CK
    nitems = nqb * _H
    hp = dh // 2

    cp_x = pltpu.make_async_copy(x_hbm, x_v, sems.at[0])
    cp_wqkv = pltpu.make_async_copy(wqkv_hbm, wqkv_v, sems.at[1])
    cp_wo = pltpu.make_async_copy(wo_hbm, wo_v, sems.at[2])
    cp_w1 = pltpu.make_async_copy(w1_hbm, w1_v, sems.at[3])
    cp_b1 = pltpu.make_async_copy(b1_hbm, b1_v, sems.at[4])
    cp_w2 = pltpu.make_async_copy(w2_hbm, w2_v, sems.at[5])

    cp_x.start()
    cp_wqkv.start()
    cp_x.wait()
    cp_wqkv.wait()
    for c in (cp_w1, cp_b1, cp_w2, cp_wo):
        c.start()
    qscale = (dh ** -0.5) * math.log2(math.e)

    def proj(i, carry):
        r0 = pl.multiple_of(i * RB, RB)
        rows = pl.ds(r0, RB)
        rows2 = pl.ds(pl.multiple_of(i * (RB // 2), RB // 2), RB // 2)
        x = x_v[rows, :].astype(F32)
        mu = jnp.mean(x, axis=-1, keepdims=True)
        xc = x - mu
        var = jnp.mean(xc * xc, axis=-1, keepdims=True)
        xn = (xc * lax.rsqrt(var + _EPS)).astype(BF16)
        xn_s[rows2, :] = _pack(xn)
        q = jnp.dot(xn, wqkv_v[:, 0:D], preferred_element_type=F32) * qscale
        qt_s[i] = _pack(q.T.astype(BF16))
        v = jnp.dot(xn, wqkv_v[:, 2 * D:3 * D], preferred_element_type=F32)
        vt_s[i] = _pack(v.T.astype(BF16))
        k = jnp.dot(xn, wqkv_v[:, D:2 * D], preferred_element_type=F32)
        for g in range(ng):
            k_s[g, rows2, :] = _pack(k[:, g * _LANES:(g + 1) * _LANES].astype(BF16))
        return carry

    lax.fori_loop(0, S // RB, proj, 0)

    assert RB == TQ

    def stage_q(t, slot, clear):
        if clear:
            prev = lax.rem(t - 2, hpg)
            qm_s[slot][pl.ds(pl.multiple_of(prev * hp, hp), hp), :] = jnp.zeros((hp, TQ), U32)
        h = lax.rem(t, _H)
        qb = jnp.minimum(lax.div(t, _H), nqb - 1)
        r = pl.multiple_of(lax.rem(t, hpg) * hp, hp)
        qm_s[slot][pl.ds(r, hp), :] = qt_s[qb, pl.ds(pl.multiple_of(h * hp, hp), hp), :]

    NG = CK // G

    def stream(t0, par, n_qk, n_pv, qk0, state):
        m_done = {0: state[0]}
        m_acc = state[1]
        hist = []
        keep = lax.broadcasted_iota(jnp.int32, (8, _LANES), 1) + t0 >= 0
        keep = jnp.concatenate([keep] * (TQ // _LANES), axis=1)
        m_cur = l_acc = o_acc = None
        for k in range(max(n_qk, n_pv)):
            if k < n_qk:
                it, j = divmod(k + qk0, nch)
                t = t0 + it
                b = (par + it) % 2
                g = lax.div(lax.rem(t, _H), hpg)
                kk = _unpack(k_s[g, j * CK // 2:(j + 1) * CK // 2, :])
                s = jnp.dot(kk, _unpack(qm_s[b][...]), preferred_element_type=F32)
                s_s[b][j * CK:(j + 1) * CK, :] = s
                m = _vreg_max(s)
                m_acc = m if j == 0 else jnp.maximum(m_acc, m)
                for r in range(NG):
                    hist.append(s[r * G + G - 8:r * G + G, :])
                if j == nch - 1:
                    m_done[it] = m_acc
                    stage_q(t + 2, b, True)
            if k < n_pv:
                it, j = divmod(k, nch)
                t = t0 + it
                b = (par + it) % 2
                h = lax.rem(t, _H)
                if j == 0:
                    m_cur = jnp.broadcast_to(jnp.max(m_done[it], axis=0, keepdims=True), (8, TQ))
                ps = [None] * NG
                for i in range(NG):
                    r = NG - 1 - i
                    mj = m_cur
                    idx = k * NG + i - FENCE
                    if FENCE and 0 <= idx < len(hist):
                        mj = jnp.where(keep, m_cur, hist[idx])
                    s = s_s[b][j * CK + r * G:j * CK + (r + 1) * G, :]
                    p = jnp.exp2(s.reshape(G // 8, 8, TQ) - mj[None])
                    l = jnp.sum(p, axis=0)
                    l_acc = l if (j == 0 and i == 0) else l_acc + l
                    ps[r] = p.reshape(G, TQ)
                blk, off = divmod(j * CK, RB)
                vt = _unpack(vt_s[blk, pl.ds(pl.multiple_of(h * hp, hp), hp), off:off + CK])
                o = jnp.dot(vt, jnp.concatenate(ps, axis=0).astype(BF16), preferred_element_type=F32)
                o_acc = o if j == 0 else o_acc + o
                if j == nch - 1:
                    qb = lax.div(t, _H)
                    ot_s[qb, pl.ds(pl.multiple_of(h * dh, dh), dh), :] = o_acc
                    l_s[qb, pl.ds(pl.multiple_of(h * 8, 8), 8), :] = l_acc
        return m_done.get(n_pv // nch), m_acc

    for t in range(2):
        qm_s[t][...] = jnp.zeros(qm_s[t].shape, U32)
        stage_q(t, t, False)
    state = stream(0, 0, nch + LAG, 0, 0, (None, None))

    def body(i, state):
        return stream(i * UNROLL, 0, UNROLL * nch, UNROLL * nch, nch + LAG, state)

    assert UNROLL % 2 == 0
    nloop = (nitems - 1) // UNROLL
    state = lax.fori_loop(0, nloop, body, state)
    t_rest = nloop * UNROLL
    n_rest = (nitems - t_rest) * nch
    stream(t_rest, 0, n_rest - nch - LAG, n_rest, nch + LAG, state)

    cp_w1.wait()
    cp_b1.wait()
    cp_w2.wait()
    cp_wo.wait()

    def out_copy(i):
        rows = pl.ds(pl.multiple_of(i * OB, OB), OB)
        return pltpu.make_async_copy(out_v.at[rows, :], out_hbm.at[rows, :], osems.at[i])

    def tail(i):
        rows = pl.ds(pl.multiple_of(i * OB, OB), OB)
        rows2 = pl.ds(pl.multiple_of(i * (OB // 2), OB // 2), OB // 2)
        xn = _unpack(xn_s[rows2, :])
        acc = x_v[rows, :].astype(F32)
        for f0 in range(0, F, FB):
            fs = slice(f0, f0 + FB)
            hh = jnp.dot(xn, w1_v[:, fs], preferred_element_type=F32) + b1_v[:, fs].astype(F32)
            sp = jnp.log1p(jnp.exp(-jnp.abs(hh))) + jnp.maximum(hh, 0.0)
            act = (hh * jnp.tanh(sp)).astype(BF16)
            acc = acc + jnp.dot(act, w2_v[fs, :], preferred_element_type=F32)
        l = jnp.sum(l_s[i].reshape(_H, 8, OB), axis=1, keepdims=True)
        o = (ot_s[i].reshape(_H, dh, OB) / l).reshape(D, OB)
        acc = acc + jnp.dot(o.T.astype(BF16), wo_v[...], preferred_element_type=F32)
        out_v[rows, :] = acc.astype(out_v.dtype)
        out_copy(i).start()

    assert OB == TQ
    tail(0)

    def tail_body(i, c):
        tail(i)
        return c

    lax.fori_loop(1, S // OB, tail_body, 0)
    for i in range(S // OB):
        out_copy(i).wait()


def make(TQ=512, CK=128, UNROLL=2, FB=256, FENCE=10, G=16, LAG=1, flags=None):
    RB = OB = TQ

    @jax.jit
    def fn(A_x, A_wqkv, A_wo, B_x, B_w1, B_b1, B_w2):
        del B_x
        B, S, D = A_x.shape
        F = B_w1.shape[1]
        assert B == 1
        ng = D // _LANES
        any_spec = pl.BlockSpec(memory_space=pl.ANY)
        out = pl.pallas_call(
            functools.partial(_kernel, S=S, D=D, F=F, TQ=TQ, CK=CK, RB=RB, UNROLL=UNROLL, FB=FB, OB=OB,
                              FENCE=FENCE, G=G, LAG=LAG),
            in_specs=[any_spec] * 6,
            out_specs=any_spec,
            out_shape=jax.ShapeDtypeStruct((S, D), A_x.dtype),
            scratch_shapes=[
                pltpu.VMEM((S, D), A_x.dtype),
                pltpu.VMEM((D, 3 * D), A_wqkv.dtype),
                pltpu.VMEM((D, D), A_wo.dtype),
                pltpu.VMEM((D, F), B_w1.dtype),
                pltpu.VMEM((1, F), B_b1.dtype),
                pltpu.VMEM((F, D), B_w2.dtype),
                pltpu.VMEM((S, D), A_x.dtype),
                pltpu.VMEM((S // 2, D), U32),
                pltpu.VMEM((S // RB, D // 2, RB), U32),
                pltpu.VMEM((ng, S // 2, _LANES), U32),
                pltpu.VMEM((S // RB, D // 2, RB), U32),
                [pltpu.VMEM((_LANES // 2, TQ), U32)] * 2,
                [pltpu.VMEM((S, TQ), F32)] * 2,
                pltpu.VMEM((S // TQ, D, TQ), F32),
                pltpu.VMEM((S // TQ, _H * 8, TQ), F32),
                pltpu.SemaphoreType.DMA((6,)),
                pltpu.SemaphoreType.DMA((S // OB,)),
            ],
            compiler_params=pltpu.CompilerParams(
                vmem_limit_bytes=100 * 1024 * 1024,
                **({"flags": flags} if flags else {}),
            ),
        )(A_x.reshape(S, D), A_wqkv, A_wo, B_w1, B_b1.reshape(1, F), B_w2)
        return out.reshape(B, S, D)
    return fn


pallas_parallel_sum__mha_block__dense_activation_mish__prompt_kernel = make(UNROLL=6, FENCE=11)
```

```python
import functools
import math

import jax
import jax.numpy as jnp
from jax import lax
import jax.experimental.pallas as pl
import jax.experimental.pallas.tpu as pltpu

_H = 32
_EPS = 1e-5
_LANES = 128
_G = 16

F32 = jnp.float32
BF16 = jnp.bfloat16
U32 = jnp.uint32


def _pack(a):
    return pltpu.bitcast(a, U32)


def _unpack(a):
    return pltpu.bitcast(a, BF16)


def _vregs(a):
    return a.reshape(a.shape[0] // 8, 8, a.shape[1])


def _quads(a):
    r, c = a.shape[0] // 2, a.shape[1] // 2
    return a[:r, :c], a[:r, c:], a[r:, :c], a[r:, c:]


def _join(c11, c12, c21, c22):
    return jnp.concatenate([jnp.concatenate([c11, c12], axis=1), jnp.concatenate([c21, c22], axis=1)], axis=0)


def _strassen_lhs(a11, a12, a21, a22):
    return [t.astype(BF16) for t in (a21 + a22, a11 + a12, a22, a11, a11 + a22, a21 - a11, a12 - a22)]


def _strassen_rhs(b11, b12, b21, b22):
    return [t.astype(BF16) for t in (b11, b22, b21 - b11, b12 - b22, b11 + b22, b11 + b12, b21 + b22)]


def _strassen_out(m2, m5, m4, m3, m1, m6, m7):
    return m4 - m5 + m1 + m7, m5 + m3, m2 + m4, m3 - m2 + m1 + m6


def _mm(a, b):
    return jnp.dot(a, b, preferred_element_type=F32)


def _kernel(x_hbm, wqkv_hbm, wo_hbm, w1_hbm, b1_hbm, w2_hbm, out_hbm,
            x_v, wqkv_v, wo_v, w1_v, b1_v, w2_v, out_v,
            xa_s, wq_s, w1_s, w2_s, wo_s, y_s,
            qt_s, k_s, vt_s, qm_s, nb_s, qb_s, qf_s, kf_s, qn_s, kn_s, ot_s, kb_s, fence_s, sems, osems,
            *, S, D, F, TQ, CK, FB, NV, VF, SH, KS, KD, QE, HPI, CB, PF32):
    RB = TQ
    dh = D // _H
    hpg = _LANES // dh
    ng = D // _LANES
    nqb = S // TQ
    nch = S // CK
    nitems = nqb * _H
    hp = dh // 2
    NG = CK // _G
    vbase = [j * NV // nch for j in range(nch + 1)]
    nvc = [vbase[j + 1] - vbase[j] for j in range(nch)]
    vgroups = [j * NG + NG - nvc[j] + v for j in range(nch) for v in range(nvc[j])]

    cp_x = [pltpu.make_async_copy(x_hbm.at[i * RB:(i + 1) * RB], x_v.at[i * RB:(i + 1) * RB], sems.at[i])
            for i in range(nqb)]
    cp_w = [pltpu.make_async_copy(wqkv_hbm.at[:, c * D:(c + 1) * D], wqkv_v.at[c], sems.at[nqb + c])
            for c in range(3)]
    cp_wo, cp_w1, cp_b1, cp_w2 = [
        pltpu.make_async_copy(src, dst, sems.at[nqb + 3 + n])
        for n, (src, dst) in enumerate([(wo_hbm, wo_v), (w1_hbm, w1_v), (b1_hbm, b1_v), (w2_hbm, w2_v)])]
    qscale = (dh ** -0.5) * math.log2(math.e)

    def head_norm2(at):
        sq = (at * at).reshape(_H, dh // 8, 8, at.shape[1])
        return jnp.sum(jnp.sum(sq, axis=1), axis=1, keepdims=True)

    todo = []

    def run_todo(n):
        for _ in range(min(n, len(todo))):
            todo.pop(0)()

    def prep_rhs(dst, w):
        r, c = w.shape[0] // 2, w.shape[1] // 2

        def piece(r0, c0, c1):
            b = [w[i + r0:i + r0 + _G, j + c0:j + c1].astype(F32) for i in (0, r) for j in (0, c)]
            for n, t in enumerate(_strassen_rhs(*b)[2:]):
                dst[n, r0 // 2:(r0 + _G) // 2, c0:c1] = _pack(t)

        return [functools.partial(piece, r0, c0, min(c0 + 256, c))
                for c0 in range(0, c, 256) for r0 in range(r - _G, -1, -_G)]

    def rhs(dst, w, n, r0, r1, c0, c1):
        if n < 2:
            r, c = n * (w.shape[0] // 2), n * (w.shape[1] // 2)
            return w[r + r0:r + r1, c + c0:c + c1]
        return _unpack(dst[n - 2, r0 // 2:r1 // 2, c0:c1])

    def layernorm(i):
        def piece(r0):
            x = jnp.concatenate([x_v[i * RB + t + r0:i * RB + t + r0 + _G, :] for t in (0, RB // 2)], axis=0)
            x = x.astype(F32)
            xc = x - jnp.mean(x, axis=-1, keepdims=True)
            var = jnp.mean(xc * xc, axis=-1, keepdims=True)
            for n, t in enumerate(_strassen_lhs(*_quads(xc * lax.rsqrt(var + _EPS)))):
                xa_s[i, n, r0 // 2:(r0 + _G) // 2, :] = _pack(t)

        return [functools.partial(piece, r0) for r0 in range(0, RB // 2, _G)]

    def project(i, c, rate):
        ms = []
        for n in range(7):
            ms.append(_mm(_unpack(xa_s[i, n]), rhs(wq_s.at[c], wqkv_v.at[c], n, 0, D // 2, 0, D // 2)))
            run_todo(rate)
        return _join(*_strassen_out(*ms))

    def proj_k(i, kn, rate):
        k = project(i, 1, rate)
        low = lax.broadcasted_iota(jnp.int32, (RB, _LANES), 1) < _LANES // 2
        rows2 = slice(i * RB // 2, (i + 1) * RB // 2)
        for g in range(ng):
            kg = k[:, g * _LANES:(g + 1) * _LANES]
            k_s[2 * g, rows2, :] = _pack(jnp.where(low, kg, 1.0).astype(BF16))
            k_s[2 * g + 1, rows2, :] = _pack(jnp.where(low, 1.0, kg).astype(BF16))
        kn2 = head_norm2(k.T)
        for c in range(0, RB, _LANES):
            kn = jnp.maximum(kn, kn2[:, :, c:c + _LANES])
        return kn

    def proj_q(i, rate):
        qt = (project(i, 0, rate) * qscale).T
        qt_s[i] = _pack(qt.astype(BF16))
        if NV:
            qf_s[i] = qt.reshape(_H, dh, RB)
        qn_s[i] = jnp.broadcast_to(head_norm2(qt), (_H, 8, RB))

    def proj_v(i, rate):
        vt = project(i, 2, rate).T
        vt_s[i] = vt if PF32 else _pack(vt.astype(BF16))

    fence_s[0] = 0

    def group(r):
        return pl.ds(pl.multiple_of(lax.rem(r, hpg) * hp, hp), hp)

    def share_of_bound(h, qb):
        kmax = jnp.concatenate([kn_s[h]] * (TQ // _LANES), axis=1)
        return (jnp.sqrt(qn_s[qb, h] * kmax) * (-1.02 / dh)).astype(BF16).astype(F32)

    def stage_q(h, qb, clear):
        if clear:
            qm_s[qb][group(h + hpg - 1), :] = jnp.zeros((hp, TQ), U32)
            qm_s[qb][group(h + hpg // 2 - 1), :] = jnp.zeros((hp, TQ), U32)
        hc = jnp.minimum(h, _H - 1)
        qm_s[qb][group(h), :] = qt_s[qb, pl.ds(pl.multiple_of(hc * hp, hp), hp), :]
        share = share_of_bound(hc, qb)
        nb_s[qb][...] = share * dh
        share = jnp.concatenate([share] * (dh // 8), axis=0)
        qm_s[qb][group(h + hpg // 2), :] = _pack(share.astype(BF16))

    def stage_v(h, qb, d0, d1, delay=lambda t: t):
        r0 = d0 // 8 * 8
        q = delay(qf_s[qb, jnp.minimum(h, _H - 1), r0:r0 + 8, :])
        for d in range(d0, d1):
            qb_s[qb % 2][d] = jnp.broadcast_to(q[d - r0:d - r0 + 1], (8, TQ))

    def stage_kf(h):
        hc = jnp.minimum(h, _H - 1)
        kk = jnp.concatenate(
            [k_s[lax.div(hc, hpg // 2), r * _G // 2:(r + 1) * _G // 2, :] for r in vgroups], axis=0)
        kf_s[...] = pltpu.roll(_unpack(kk).astype(F32), lax.rem(hpg - lax.rem(hc, hpg), hpg) * dh, 1)

    def stage_k(par, d, v0, v1, delay=lambda t: t):
        kv = delay(kf_s[v0 * _G:v1 * _G, :])
        kb_s[par][d, v0 * _G:v1 * _G, :] = jnp.broadcast_to(kv[:, d:d + 1], kv.shape)

    cp_x[0].start()
    cp_w[1].start()
    for qb in range(nqb):
        qm_s[qb][...] = jnp.zeros(qm_s[qb].shape, U32)
    cp_x[0].wait()
    for c in (cp_w[0], cp_w[2], cp_x[1]):
        c.start()
    cp_w[1].wait()
    todo += layernorm(0)
    run_todo(len(todo))
    todo += prep_rhs(wq_s.at[1], wqkv_v.at[1])
    kn = proj_k(0, jnp.zeros((_H, 1, _LANES), F32), 8)
    for c in (cp_w[0], cp_w[2], cp_x[1]):
        c.wait()
    for c in cp_x[2:] + [cp_w1, cp_b1, cp_w2, cp_wo]:
        c.start()
    todo += prep_rhs(wq_s.at[0], wqkv_v.at[0])
    proj_q(0, 8)
    todo += prep_rhs(wq_s.at[2], wqkv_v.at[2]) + layernorm(1)
    proj_v(0, 8)
    for i in range(1, nqb):
        if i == 1:
            for c in cp_x[2:]:
                c.wait()
        if i == 2:
            for c in (cp_w1, cp_b1, cp_w2, cp_wo):
                c.wait()
            todo += prep_rhs(w1_s, w1_v) + prep_rhs(w2_s, w2_v) + prep_rhs(wo_s, wo_v)
        if i + 1 < nqb:
            todo[:0] = layernorm(i + 1)
        kn = proj_k(i, kn, 1 if i == 1 else 4)
        if i + 1 == nqb:
            kn_s[...] = jnp.broadcast_to(jnp.max(kn, axis=2, keepdims=True), kn_s.shape)
            if NV:
                todo[:0] = [functools.partial(stage_kf, 0)] + [
                    functools.partial(stage_k, 0, d, 0, NV) for d in range(dh)]
        proj_q(i, 1 if i == 1 else 4)
        if i + 1 == nqb:
            todo += [functools.partial(stage_q, 0, qb, False) for qb in range(nqb)]
            todo += [functools.partial(stage_v, 0, 0, d, d + 8) for d in range(0, dh, 8)]
        proj_v(i, 1 if i == 1 else 4)
    run_todo(len(todo))

    def mish(hh):
        e = jnp.exp(jnp.minimum(hh, 30.0))
        n = e * (e + 2.0)
        den = n + 2.0
        r = pl.reciprocal(den, approx=True)
        return hh * (n * (r * (2.0 - den * r)))

    def ffn(i, c):
        b1 = b1_v[...].astype(F32).reshape(1, F)
        spans = [(f0, min(f0 + FB, F // 2)) for f0 in range(0, F // 2, FB)]
        acts, acc = [], None
        for n_ in range(len(spans) + 1):
            if n_ < len(spans):
                f0, f1 = spans[n_]
                hs = _strassen_out(*[_mm(_unpack(xa_s[i, n]), rhs(w1_s, w1_v, n, 0, D // 2, f0, f1)) for n in range(7)])
                bs = (b1[:, f0:f1], b1[:, F // 2 + f0:F // 2 + f1]) * 2
                acts.append(_strassen_lhs(*[mish(t + b) for t, b in zip(hs, bs)]))
            if n_ > 0:
                f0, f1 = spans[n_ - 1]
                ms = [_mm(acts[n_ - 1][n], rhs(w2_s, w2_v, n, f0, f1, 0, D // 2)) for n in range(7)]
                acc = ms if acc is None else [t + m for t, m in zip(acc, ms)]
        x = x_v[pl.ds(pl.multiple_of(i * RB, RB), RB), :].astype(F32)
        y_s[i] = x + _join(*_strassen_out(*acc))
        return c

    lax.fori_loop(0, nqb, ffn, 0)

    mseq = [j * NG + r for j in range(nch) for r in reversed(range(NG - nvc[j]))]
    cuts = [0] + [(j + 1) * NG - vbase[j + 1] + SH for j in range(nch - 1)] + [len(mseq)]
    nslot = len(mseq) + nch
    nstep = NV * dh

    def stream(h0, n_qk, n_pv, qk0, state):
        pm, pv, acc, l_acc, (lo, hi) = list(state[0]), list(state[1]), state[2], state[3], state[4]
        o_acc = None
        l_done = {}
        hist = []
        due = []
        keep = lax.broadcasted_iota(jnp.int32, (8, _LANES), 1) + h0 >= 0
        zero = fence_s[0]
        keep2 = lax.broadcasted_iota(jnp.int32, (8, _LANES), 0) + zero >= 0
        steps_before = lambda c: (c // nch) * nstep + (c % nch) * nstep // nch
        u0 = steps_before(qk0)

        def finish(s, first):
            nonlocal l_acc
            p = jnp.exp2(s)
            l_acc = p[:8] if first else l_acc + p[:8]
            l_acc = l_acc + p[8:]
            return p

        for k in range(max(n_qk, n_pv)):
            if k < n_qk:
                it, j = divmod(k + qk0, nch)
                hi_, qb = divmod(it, nqb)
                h = h0 + hi_
                hc = jnp.minimum(h, _H - 1)
                groups = mseq[cuts[j]:cuts[j + 1]]
                kg = lax.div(hc, hpg // 2)
                kk = jnp.concatenate([k_s[kg, r * _G // 2:(r + 1) * _G // 2, :] for r in groups], axis=0)
                qm = qm_s[qb][pl.ds(pl.multiple_of(zero, 8), _LANES // 2), :]
                s = jnp.dot(_unpack(kk), _unpack(qm), preferred_element_type=F32)
                for n in range(len(groups)):
                    hist.append(s[(n + 1) * _G - 8:(n + 1) * _G, :_LANES])
                    pm.append(finish(s[n * _G:(n + 1) * _G], j == 0 and n == 0))
                for u in range(steps_before(k + qk0), steps_before(k + qk0 + 1)):
                    v, d = divmod(u % nstep, dh)
                    if d == 0:
                        acc = nb_s[qb][pl.ds(pl.multiple_of(zero, 8), 8), :][None]
                    kb = _vregs(kb_s[hi_ % 2][d + zero, v * _G:(v + 1) * _G, :])
                    idx = (u - u0) * nslot // nstep - VF
                    if idx >= 0:
                        after = hist[idx]
                        while due:
                            after = jnp.where(keep2, after, due.pop())
                        kb = jnp.where(keep[None], kb, after[None])
                    kb = jnp.concatenate([kb] * (TQ // _LANES), axis=2)
                    acc = acc + kb * qb_s[qb % 2][d + zero][None]
                    if d == dh - 1:
                        pv.append(finish(acc.reshape(_G, TQ), False))
                        acc = None
                if j == nch - 1:
                    lt = jnp.sum(l_acc, axis=0, keepdims=True)
                    lo = jnp.minimum(lo, lt)
                    hi = hi + lt
                    l_done[it] = 1.0 / lt
                    stage_q(h + 1, qb, True)
                def delay(t):
                    t3 = _vregs(t)
                    after = hist[max(len(hist) - KD, 0)]
                    after = jnp.concatenate([after] * (t.shape[1] // _LANES), axis=1)
                    mask = jnp.concatenate([keep] * (t.shape[1] // _LANES), axis=1)
                    return jnp.where(mask[None], t3, after[None]).reshape(t.shape)

                if NV and j % QE == QE // 2:
                    d0 = j // QE * QE * dh // nch
                    stage_v(h + (qb + 1) // nqb, (qb + 1) % nqb, d0, d0 + QE * dh // nch, delay)
                    due.append(qb_s[(qb + 1) % 2][d0 + zero, :, :_LANES])
                if NV and n_pv:
                    hk, kk_ = divmod(k, nqb * nch)
                    span = nqb * nch - qk0 - 1
                    parts = dh * KS
                    if kk_ == 0:
                        stage_kf(h0 + hk + 1)
                    else:
                        for u in range((kk_ - 1) * parts // span, min(kk_ * parts // span, parts)):
                            v0 = (u % KS) * NV // KS
                            stage_k((hk + 1) % 2, u // KS, v0, (u % KS + 1) * NV // KS, delay)
                            due.append(kb_s[(hk + 1) % 2][u // KS + zero, v0 * _G:v0 * _G + 8, :])
            if k < n_pv:
                it, j = divmod(k, nch)
                hi_, qb = divmod(it, nqb)
                h = h0 + hi_
                parts = [pm.pop(0) for _ in range(NG - nvc[j])][::-1] + [pv.pop(0) for _ in range(nvc[j])]
                p = jnp.concatenate([t.astype(F32) for t in parts], axis=0)
                blk, off = divmod(j * CK, RB)
                if PF32:
                    vt = vt_s[blk, pl.ds(pl.multiple_of(h * dh, dh), dh), off:off + CK]
                    o = jnp.dot(vt, p, preferred_element_type=F32)
                else:
                    vt = _unpack(vt_s[blk, pl.ds(pl.multiple_of(h * hp, hp), hp), off:off + CK])
                    o = jnp.dot(vt, p.astype(BF16), preferred_element_type=F32)
                hist.append(o[8:, :_LANES])
                o_acc = o if j == 0 else o_acc + o
                if j == nch - 1:
                    ot_s[qb, pl.ds(pl.multiple_of(h * dh, dh), dh), :] = o_acc * l_done[it]
        cast = (lambda t: t.astype(BF16)) if CB else (lambda t: t)
        return tuple(map(cast, pm)), tuple(map(cast, pv)), acc, l_acc, (lo, hi)

    state = stream(0, 1, 0, 0, ((), (), None, None, (jnp.full((1, TQ), 1.0, F32), jnp.zeros((1, TQ), F32))))

    def body(i, state):
        return stream(i * HPI, HPI * nqb * nch, HPI * nqb * nch, 1, state)

    assert HPI % 2 == 0
    state = lax.fori_loop(0, _H // HPI, body, state)
    lo, hi = state[4]

    safe = jnp.where((lo >= 2.0 ** -64) & (hi <= 2.0 ** 40), 1.0, 0.0)

    @pl.when(jnp.min(safe) < 0.5)
    def _():
        def item(t, c):
            h = lax.rem(t, _H)
            qb = lax.div(t, _H)
            kg = lax.div(h, hpg // 2)
            qm_s[0][...] = jnp.zeros(qm_s[0].shape, U32)
            qm_s[0][group(t), :] = qt_s[qb, pl.ds(pl.multiple_of(h * hp, hp), hp), :]

            def scores(blk):
                kk = k_s[kg, pl.ds(pl.multiple_of(blk * (RB // 2), RB // 2), RB // 2), :]
                return jnp.dot(_unpack(kk), _unpack(qm_s[0][...]), preferred_element_type=F32)

            def max_step(blk, m):
                return jnp.maximum(m, jnp.max(scores(blk), axis=0, keepdims=True))

            m = lax.fori_loop(0, S // RB, max_step, jnp.full((1, TQ), -jnp.inf, F32))

            def pv_step(blk, lo_):
                p = jnp.exp2(scores(blk) - m)
                if PF32:
                    vt = vt_s[blk, pl.ds(pl.multiple_of(h * dh, dh), dh), :].astype(BF16)
                else:
                    vt = _unpack(vt_s[blk, pl.ds(pl.multiple_of(h * hp, hp), hp), :])
                o = jnp.dot(vt, p.astype(BF16), preferred_element_type=F32)
                return lo_[0] + jnp.sum(p, axis=0, keepdims=True), lo_[1] + o

            l, o = lax.fori_loop(0, S // RB, pv_step, (jnp.zeros((1, TQ), F32), jnp.zeros((dh, TQ), F32)))
            ot_s[qb, pl.ds(pl.multiple_of(h * dh, dh), dh), :] = o / l
            return c

        lax.fori_loop(0, nitems, item, 0)

    cp_out = [pltpu.make_async_copy(out_v.at[i * RB:(i + 1) * RB], out_hbm.at[i * RB:(i + 1) * RB], osems.at[i])
              for i in range(nqb)]
    for i in range(nqb):
        lhs = _strassen_lhs(*_quads(ot_s[i].T))
        proj = _join(*_strassen_out(*[_mm(lhs[n], rhs(wo_s, wo_v, n, 0, D // 2, 0, D // 2)) for n in range(7)]))
        out_v[i * RB:(i + 1) * RB, :] = (y_s[i] + proj).astype(out_v.dtype)
        cp_out[i].start()
    for c in cp_out:
        c.wait()


def make(TQ=512, CK=128, FB=256, NV=14, VF=8, SH=2, KS=1, KD=24, QE=2, HPI=2, CB=1, PF32=False, flags=None):
    @jax.jit
    def fn(A_x, A_wqkv, A_wo, B_x, B_w1, B_b1, B_w2):
        del B_x
        B, S, D = A_x.shape
        F = B_w1.shape[1]
        assert B == 1
        ng = D // _LANES
        dh = D // _H
        any_spec = pl.BlockSpec(memory_space=pl.ANY)
        out = pl.pallas_call(
            functools.partial(_kernel, S=S, D=D, F=F, TQ=TQ, CK=CK, FB=FB,
                              NV=NV, VF=VF, SH=SH, KS=KS, KD=KD, QE=QE, HPI=HPI, CB=CB, PF32=PF32),
            in_specs=[any_spec] * 6,
            out_specs=any_spec,
            out_shape=jax.ShapeDtypeStruct((S, D), A_x.dtype),
            scratch_shapes=[
                pltpu.VMEM((S, D), A_x.dtype),
                pltpu.VMEM((3, D, D), A_wqkv.dtype),
                pltpu.VMEM((D, D), A_wo.dtype),
                pltpu.VMEM((D, F), B_w1.dtype),
                pltpu.VMEM((F,), B_b1.dtype),
                pltpu.VMEM((F, D), B_w2.dtype),
                pltpu.VMEM((S, D), A_x.dtype),
                pltpu.VMEM((S // TQ, 7, TQ // 4, D // 2), U32),
                pltpu.VMEM((3, 5, D // 4, D // 2), U32),
                pltpu.VMEM((5, D // 4, F // 2), U32),
                pltpu.VMEM((5, F // 4, D // 2), U32),
                pltpu.VMEM((5, D // 4, D // 2), U32),
                pltpu.VMEM((S // TQ, TQ, D), F32),
                pltpu.VMEM((S // TQ, D // 2, TQ), U32),
                pltpu.VMEM((2 * ng, S // 2, _LANES), U32),
                pltpu.VMEM((S // TQ, D, TQ), F32) if PF32 else pltpu.VMEM((S // TQ, D // 2, TQ), U32),
                [pltpu.VMEM((_LANES // 2, TQ), U32)] * (S // TQ),
                [pltpu.VMEM((8, TQ), F32)] * (S // TQ),
                [pltpu.VMEM((dh, 8, TQ), F32)] * 2,
                pltpu.VMEM((S // TQ, _H, dh, TQ), F32),
                pltpu.VMEM((max(NV, 1) * _G, _LANES), F32),
                pltpu.VMEM((S // TQ, _H, 8, TQ), F32),
                pltpu.VMEM((_H, 8, _LANES), F32),
                pltpu.VMEM((S // TQ, D, TQ), F32),
                [pltpu.VMEM((dh, max(NV, 1) * _G, _LANES), F32)] * 2,
                pltpu.SMEM((3,), jnp.int32),
                pltpu.SemaphoreType.DMA((S // TQ + 7,)),
                pltpu.SemaphoreType.DMA((S // TQ,)),
            ],
            compiler_params=pltpu.CompilerParams(
                vmem_limit_bytes=100 * 1024 * 1024,
                **({"flags": flags} if flags else {}),
            ),
        )(A_x.reshape(S, D), A_wqkv, A_wo, B_w1, B_b1, B_w2)
        return out.reshape(B, S, D)
    return fn


pallas_parallel_sum__mha_block__dense_activation_mish__prompt_kernel = make(KS=4, QE=4)
```

```python
import functools
import math

import jax
import jax.numpy as jnp
from jax import lax
import jax.experimental.pallas as pl
import jax.experimental.pallas.tpu as pltpu

_H = 32
_EPS = 1e-5
_LANES = 128
_G = 16
_TQ = 512
_CK = 128

F32 = jnp.float32
BF16 = jnp.bfloat16
U32 = jnp.uint32


def _pack(a):
    return pltpu.bitcast(a, U32)


def _unpack(a):
    return pltpu.bitcast(a, BF16)


def _vregs(a):
    return a.reshape(a.shape[0] // 8, 8, a.shape[1])


def _widen(a, width):
    return jnp.concatenate([a] * (width // a.shape[-1]), axis=-1)


def _mm(a, b):
    return jnp.dot(a, b, preferred_element_type=F32)


def _recip(a):
    r = pl.reciprocal(a, approx=True)
    return r * (2.0 - a * r)


def _mish(h):
    e = jnp.exp(jnp.minimum(h, 30.0))
    n = e * (e + 2.0)
    return h * (n * _recip(n + 2.0))


def _quads(a):
    r, c = a.shape[0] // 2, a.shape[1] // 2
    return a[:r, :c], a[:r, c:], a[r:, :c], a[r:, c:]


def _join(c11, c12, c21, c22):
    return jnp.concatenate([jnp.concatenate([c11, c12], axis=1), jnp.concatenate([c21, c22], axis=1)], axis=0)


def _strassen_lhs(a11, a12, a21, a22):
    return [t.astype(BF16) for t in (a21 + a22, a11 + a12, a22, a11, a11 + a22, a21 - a11, a12 - a22)]


def _strassen_rhs(b11, b12, b21, b22):
    f11, f12, f21, f22 = [t.astype(F32) for t in (b11, b12, b21, b22)]
    return [b11, b22] + [t.astype(BF16) for t in (f21 - f11, f12 - f22, f11 + f22, f11 + f12, f21 + f22)]


def _strassen_out(m2, m5, m4, m3, m1, m6, m7):
    return m4 - m5 + m1 + m7, m5 + m3, m2 + m4, m3 - m2 + m1 + m6


def _quad_slices(w_ref, r0, r1, c0, c1):
    r, c = w_ref.shape[0] // 2, w_ref.shape[1] // 2
    return [w_ref[i + r0:i + r1, j + c0:j + c1] for i in (0, r) for j in (0, c)]


def _not_before(true_mask, token):
    def delay(t):
        if token is None:
            return t
        width = t.shape[1]
        return jnp.where(_widen(true_mask, width)[None], _vregs(t), _widen(token, width)[None]).reshape(t.shape)
    return delay


def _kernel(x_hbm, wqkv_hbm, wo_hbm, w1_hbm, b1_hbm, w2_hbm, out_hbm,
            x_v, wqkv_v, wo_v, w1_v, b1_v, w2_v, out_v,
            xa_s, wq_s, y_s, qt_s, k_s, vt_s, qn_s, kn_s, kf_s,
            qm_s, shift_s, qb_s, kb_s, ot_s, l_s, zero_s, in_sems, out_sems,
            *, FB, SH, VF, VG, KS, KD, KE, KN, QE, WA, WB):
    S, D = x_v.shape
    F = w1_v.shape[1]
    dh = D // _H
    hp = dh // 2
    hpg = _LANES // dh
    nqb = S // _TQ
    nch = S // _CK
    ng = _CK // _G

    zero_s[0] = 0
    always = lax.broadcasted_iota(jnp.int32, (8, _LANES), 0) + zero_s[0] >= 0

    def rows_of(i, n):
        return pl.ds(pl.multiple_of(i * n, n), n)

    def clamp(h):
        return jnp.minimum(h, _H - 1)

    def stage_q(h, qb, clear):
        if clear:
            qm_s[qb][rows_of(lax.rem(h + hpg - 1, hpg), hp), :] = jnp.zeros((hp, _TQ), U32)
            qm_s[qb][rows_of(lax.rem(h + hpg // 2 - 1, hpg), hp), :] = jnp.zeros((hp, _TQ), U32)
        qm_s[qb][rows_of(lax.rem(h, hpg), hp), :] = qt_s[qb, rows_of(clamp(h), hp), :]
        norm2 = qn_s[qb, clamp(h)] * _widen(kn_s[clamp(h)], _TQ)
        bound = jnp.exp2(jnp.log(norm2) * (0.5 / math.log(2.0))) * 1.02
        share = (bound * (-1.0 / dh)).astype(BF16).astype(F32)
        shift_s[qb][...] = share * dh
        qm_s[qb][rows_of(lax.rem(h + hpg // 2, hpg), hp), :] = _pack(
            jnp.concatenate([share] * (dh // 8), axis=0).astype(BF16))

    def stage_qb(h, qb, d0, d1, delay):
        r0 = d0 // 8 * 8
        q = delay(_unpack(qt_s[qb, rows_of(clamp(h), hp), :]).astype(F32)[r0:r0 + 8])
        for d in range(d0, d1):
            qb_s[qb % 2][d] = jnp.broadcast_to(q[d - r0:d - r0 + 1], (8, _TQ))

    def stage_kb(h, slot, d, v0, v1, delay):
        k = kf_s[clamp(h), v0 * _G:v1 * _G, :]
        k = jnp.concatenate([delay(k[:KN * 8]), k[KN * 8:]], axis=0)
        kb_s[slot][d, v0 * _G:v1 * _G, :] = jnp.broadcast_to(k[:, d:d + 1], k.shape)

    todo = []

    def run_todo(n, after=None):
        n = min(n, len(todo))
        for u in range(n):
            r = 0 if after is None else u * (after.shape[0] // 8) // n * 8
            todo.pop(0)(_not_before(always, None if after is None else after[r:r + 8, :_LANES]))

    def weight_pieces(c):
        def piece(r0, delay):
            b = [delay(t.astype(F32)) for t in _quad_slices(wqkv_v.at[c], r0, r0 + _G, 0, D // 2)]
            for n, t in enumerate(_strassen_rhs(*b)[2:]):
                wq_s[c, n, r0 // 2:(r0 + _G) // 2, :] = _pack(t)
        return [functools.partial(piece, r0) for r0 in range(D // 2 - _G, -1, -_G)]

    def layernorm_pieces(i):
        def piece(r0, delay):
            x = [x_v[i * _TQ + t + r0:i * _TQ + t + r0 + _G, :] for t in (0, _TQ // 2)]
            x = delay(jnp.concatenate(x, axis=0).astype(F32))
            xc = x - jnp.mean(x, axis=-1, keepdims=True)
            var = jnp.mean(xc * xc, axis=-1, keepdims=True)
            for n, t in enumerate(_strassen_lhs(*_quads(xc * lax.rsqrt(var + _EPS)))):
                xa_s[i, n, r0 // 2:(r0 + _G) // 2, :] = _pack(t)
        return [functools.partial(piece, r0) for r0 in range(0, _TQ // 2, _G)]

    def project(i, c, rate, wait_at=None, copies=(), weight=None):
        raw = _quad_slices(wqkv_v.at[c], 0, D // 2, 0, D // 2)
        ms = []
        for n in range(7):
            if n == wait_at:
                for cp in copies:
                    cp.wait()
                todo.extend(weight_pieces(weight))
            ms.append(_mm(_unpack(xa_s[i, n]), raw[3 * n] if n < 2 else _unpack(wq_s[c, n - 2])))
            run_todo(rate, ms[-1])
        return _join(*_strassen_out(*ms))

    def head_sum(a):
        return jnp.sum(jnp.sum(a.reshape(_H, dh // 8, 8, a.shape[1]), axis=1), axis=1, keepdims=True)

    def project_k(i, kn, *args):
        k = project(i, 1, *args)
        low = lax.broadcasted_iota(jnp.int32, (_TQ // 2, _LANES), 1) < _LANES // 2
        ones = jnp.full(low.shape, 0x3F803F80, U32)
        for g in range(D // _LANES):
            kg = k[:, g * _LANES:(g + 1) * _LANES]
            kp = _pack(kg.astype(BF16))
            k_s[2 * g, i * _TQ // 2:(i + 1) * _TQ // 2, :] = jnp.where(low, kp, ones)
            k_s[2 * g + 1, i * _TQ // 2:(i + 1) * _TQ // 2, :] = jnp.where(low, ones, kp)
            for j in range(_TQ // _CK):
                kv = kg[(j + 1) * _CK - _G:(j + 1) * _CK]
                v = i * (_TQ // _CK) + j
                for t in range(hpg):
                    kf_s[g * hpg + t, v * _G:(v + 1) * _G, :] = pltpu.roll(kv, _LANES - t * dh, 1) if t else kv
        return jnp.maximum(kn, head_sum(jnp.max((k * k).reshape(_TQ // _LANES, _LANES, D), axis=0).T))

    def project_q(i, *args):
        qt = (project(i, 0, *args) * (dh ** -0.5 * math.log2(math.e))).T
        qt_s[i] = _pack(qt.astype(BF16))
        qn_s[i] = jnp.broadcast_to(head_sum(qt * qt), (_H, 8, _TQ))

    def project_v(i, *args):
        vt_s[i] = _pack(project(i, 2, *args).T.astype(BF16))

    cp_x = [pltpu.make_async_copy(x_hbm.at[i * _TQ:(i + 1) * _TQ], x_v.at[i * _TQ:(i + 1) * _TQ], in_sems.at[i])
            for i in range(nqb)]
    cp_q, cp_k, cp_v = [
        pltpu.make_async_copy(wqkv_hbm.at[:, c * D:(c + 1) * D], wqkv_v.at[c], in_sems.at[nqb + c])
        for c in range(3)]
    cp_rest = [pltpu.make_async_copy(src, dst, in_sems.at[nqb + 3 + n])
               for n, (src, dst) in enumerate([(w1_hbm, w1_v), (b1_hbm, b1_v), (w2_hbm, w2_v), (wo_hbm, wo_v)])]
    for cp in [cp_x[0], cp_k, cp_q, cp_x[1], cp_v] + cp_x[2:] + cp_rest:
        cp.start()
    for qb in range(nqb):
        qm_s[qb][...] = jnp.zeros(qm_s[qb].shape, U32)
    cp_x[0].wait()
    todo += layernorm_pieces(0)
    run_todo(len(todo))
    cp_k.wait()
    todo += weight_pieces(1)
    run_todo(len(todo))
    kn = project_k(0, jnp.zeros((_H, 1, _LANES), F32), 8, WA, [cp_q, cp_x[1]], 0)
    todo += layernorm_pieces(1)
    project_q(0, 3)
    kn = project_k(1, kn, 6, WB, [cp_v] + cp_x[2:], 2)
    project_v(0, 4)
    todo += layernorm_pieces(2)
    project_q(1, 1)
    project_v(1, 2)
    todo += layernorm_pieces(3)
    kn = project_k(2, kn, 1)
    project_v(2, 2)
    kn = project_k(3, kn, 0)
    kn_s[...] = jnp.broadcast_to(jnp.max(kn, axis=2, keepdims=True), kn_s.shape)
    project_q(2, 0)
    todo += [functools.partial(stage_kb, 0, 0, d, 0, nch) for d in range(dh)]
    project_q(3, 3)
    todo += [functools.partial(stage_qb, 0, 0, d, d + 8) for d in range(0, dh, 8)]
    todo += [functools.partial(lambda qb, delay: stage_q(0, qb, False), qb) for qb in range(nqb)]
    project_v(3, 6)
    for cp in cp_rest:
        cp.wait()

    b1 = b1_v[...].astype(F32).reshape(1, F)
    spans = [(f0, min(f0 + FB, F // 2)) for f0 in range(0, F // 2, FB)]

    def ffn(i, carry):
        def up(f0, f1):
            ws = _strassen_rhs(*_quad_slices(w1_v, 0, D // 2, f0, f1))
            hs = _strassen_out(*[_mm(_unpack(xa_s[i, n]), ws[n]) for n in range(7)])
            bs = (b1[:, f0:f1], b1[:, F // 2 + f0:F // 2 + f1]) * 2
            return _strassen_lhs(*[_mish(t + b) for t, b in zip(hs, bs)])

        act, acc = up(*spans[0]), None
        for u, (f0, f1) in enumerate(spans):
            nxt = up(*spans[u + 1]) if u + 1 < len(spans) else None
            ms = [_mm(a, w) for a, w in zip(act, _strassen_rhs(*_quad_slices(w2_v, f0, f1, 0, D // 2)))]
            acc = ms if u == 0 else [t + m for t, m in zip(acc, ms)]
            act = nxt
        y_s[i] = x_v[rows_of(i, _TQ), :].astype(F32) + _join(*_strassen_out(*acc))
        return carry

    lax.fori_loop(0, nqb, ffn, 0)

    order = [j * ng + r for j in range(nch) for r in reversed(range(ng - 1))]
    cuts = [j * (ng - 1) + SH for j in range(nch)] + [len(order)]

    def stream(h0, first, n_qk, n_pv, state):
        p_mxu, p_tile, l_acc, lo, hi = state
        p_mxu, p_vpu = list(p_mxu), []
        zero = zero_s[0]
        also = lax.broadcasted_iota(jnp.int32, (8, _LANES), 1) + h0 >= 0
        results = []
        staged = []

        def exp_and_sum(s, reset):
            nonlocal l_acc
            p = jnp.exp2(s)
            l_acc = p[:8] if reset else l_acc + p[:8]
            l_acc = l_acc + p[8:]
            return p

        def mxu_scores(item, g0, g1):
            kg = lax.div(clamp(h0 + item // nqb), hpg // 2)
            k = jnp.concatenate([k_s[kg, r * _G // 2:(r + 1) * _G // 2, :] for r in order[g0:g1]], axis=0)
            s = _mm(_unpack(k), _unpack(qm_s[item % nqb][rows_of(zero, _LANES // 2), :]))
            for n in range(g1 - g0):
                results.append(s[(n + 1) * _G - 8:(n + 1) * _G, :_LANES])
                p_mxu.append(exp_and_sum(s[n * _G:(n + 1) * _G], g0 + n == 0))

        def vpu_scores(item, j, slot0):
            qb = item % nqb
            acc = shift_s[qb][rows_of(zero, 8), :][None]
            for d in range(dh):
                k = kb_s[item // nqb % 2][d + zero, j * _G:(j + 1) * _G, :]
                slot = slot0 + d * ng // dh - VF
                if slot >= 0 and d % VG == 0:
                    token = results[slot]
                    while staged:
                        token = jnp.where(always, token, staged.pop())
                    k = _not_before(also, token)(k)
                acc = acc + _widen(_vregs(k), _TQ) * qb_s[qb % 2][d + zero][None]
            p_vpu.append(exp_and_sum(acc.reshape(_G, _TQ), False))

        def next_tile():
            parts = [p_mxu.pop(0) for _ in range(ng - 1)][::-1] + [p_vpu.pop(0)]
            return jnp.concatenate(parts, axis=0).astype(BF16)

        if first == 0:
            mxu_scores(0, 0, SH)
        for t in range(max(n_qk, n_pv)):
            if t < n_qk:
                item, j = divmod(first + t, nch)
                h, qb = h0 + item // nqb, item % nqb
                mxu_scores(item, cuts[j], cuts[j + 1])
                vpu_scores(item, j, t * ng)
                if j == nch - 1:
                    lo = jnp.minimum(lo, l_acc)
                    hi = hi + l_acc
                    l_s[qb, clamp(h)] = l_acc
                    stage_q(h + 1, qb, True)
                    mxu_scores(item + 1, 0, SH)
                delay = _not_before(also, results[max(len(results) - KD, 0)])
                if j % QE == QE // 2:
                    d0 = j // QE * QE * dh // nch
                    stage_qb(h + (qb + 1) // nqb, (qb + 1) % nqb, d0, d0 + QE * dh // nch, delay)
                    staged.append(qb_s[(qb + 1) % 2][d0 + zero, :, :_LANES])
                if n_pv:
                    hk, tk = divmod(t, nqb * nch)
                    span, pieces = nqb * nch - first - KE, dh * KS
                    for u in range(tk * pieces // span, min((tk + 1) * pieces // span, pieces)):
                        d, v0, v1 = u // KS, u % KS * nch // KS, (u % KS + 1) * nch // KS
                        stage_kb(h0 + hk + 1, (hk + 1) % 2, d, v0, v1, delay)
                        staged.append(kb_s[(hk + 1) % 2][d + zero, v0 * _G:v0 * _G + 8, :])
            if t < n_pv:
                item, j = divmod(t, nch)
                h = h0 + item // nqb
                blk, off = divmod(j * _CK, _TQ)
                o = _mm(_unpack(vt_s[blk, rows_of(h, hp), off:off + _CK]), next_tile() if t else p_tile)
                results.append(o[8:, :_LANES])
                o_acc = o if j == 0 else o_acc + o
                if j == nch - 1:
                    ot_s[item % nqb, rows_of(h, dh), :] = o_acc
        p_tile = next_tile()
        return tuple(p_mxu), p_tile, l_acc, lo, hi

    state = stream(0, 0, 1, 0, ((), None, None, jnp.ones((8, _TQ), F32), jnp.zeros((8, _TQ), F32)))
    n = 2 * nqb * nch
    lo, hi = lax.fori_loop(0, _H // 2, lambda i, st: stream(2 * i, 1, n, n, st), state)[3:]

    safe = jnp.where((lo >= 2.0 ** -64) & (hi <= 2.0 ** 40), 1.0, 0.0)

    @pl.when(jnp.min(safe) < 0.5)
    def _():
        def redo(t, carry):
            h, qb = lax.rem(t, _H), lax.div(t, _H)
            qm_s[0][...] = jnp.zeros(qm_s[0].shape, U32)
            qm_s[0][rows_of(lax.rem(h, hpg), hp), :] = qt_s[qb, rows_of(h, hp), :]

            def scores(blk):
                return _mm(_unpack(k_s[lax.div(h, hpg // 2), rows_of(blk, _TQ // 2), :]), _unpack(qm_s[0][...]))

            m = lax.fori_loop(0, nqb, lambda blk, m: jnp.maximum(m, jnp.max(scores(blk), axis=0, keepdims=True)),
                              jnp.full((1, _TQ), -jnp.inf, F32))

            def weigh(blk, sums):
                p = jnp.exp2(scores(blk) - m)
                o = _mm(_unpack(vt_s[blk, rows_of(h, hp), :]), p.astype(BF16))
                return sums[0] + jnp.sum(_vregs(p), axis=0), sums[1] + o

            l, o = lax.fori_loop(0, nqb, weigh, (jnp.zeros((8, _TQ), F32), jnp.zeros((dh, _TQ), F32)))
            l_s[qb, h] = l
            ot_s[qb, rows_of(h, dh), :] = o
            return carry

        lax.fori_loop(0, nqb * _H, redo, 0)

    cp_out = []

    def send(*index):
        cp_out.append(pltpu.make_async_copy(out_v.at[index], out_hbm.at[index], out_sems.at[len(cp_out)]))
        cp_out[-1].start()

    ws = _strassen_rhs(*_quad_slices(wo_v, 0, D // 2, 0, D // 2))
    for i in range(nqb):
        o = ot_s[i].reshape(_H, dh, _TQ) * _recip(jnp.sum(l_s[i], axis=1, keepdims=True))
        cs = _strassen_out(*[_mm(a, w) for a, w in zip(_strassen_lhs(*_quads(o.reshape(D, _TQ).T)), ws)])
        for u in (1, 2, 0, 3):
            r0, c0 = u // 2 * (_TQ // 2), u % 2 * (D // 2)
            rows, cols = slice(i * _TQ + r0, i * _TQ + r0 + _TQ // 2), slice(c0, c0 + D // 2)
            out_v[rows, cols] = (y_s[i, r0:r0 + _TQ // 2, cols] + cs[u]).astype(out_v.dtype)
            if i + 1 == nqb:
                send(rows, cols)
        if i + 1 < nqb:
            send(slice(i * _TQ, (i + 1) * _TQ))
    for cp in cp_out:
        cp.wait()


def make(FB=384, SH=2, VF=8, VG=2, KS=4, KD=24, KE=4, KN=1, QE=2, WA=5, WB=5, interpret=False):
    @jax.jit
    def fn(A_x, A_wqkv, A_wo, B_x, B_w1, B_b1, B_w2):
        del B_x
        B, S, D = A_x.shape
        F = B_w1.shape[1]
        dh, nqb, nch = D // _H, S // _TQ, S // _CK
        assert (B, nqb * _TQ, dh) == (1, S, _G) and nqb == 4 and F % (2 * _LANES) == 0
        hbm = pl.BlockSpec(memory_space=pl.ANY)
        vmem = pltpu.VMEM
        out = pl.pallas_call(
            functools.partial(_kernel, FB=FB, SH=SH, VF=VF, VG=VG, KS=KS, KD=KD, KE=KE, KN=KN, QE=QE, WA=WA, WB=WB),
            in_specs=[hbm] * 6,
            out_specs=hbm,
            out_shape=jax.ShapeDtypeStruct((S, D), A_x.dtype),
            scratch_shapes=[
                vmem((S, D), A_x.dtype),
                vmem((3, D, D), A_wqkv.dtype),
                vmem((D, D), A_wo.dtype),
                vmem((D, F), B_w1.dtype),
                vmem((F,), B_b1.dtype),
                vmem((F, D), B_w2.dtype),
                vmem((S, D), A_x.dtype),
                vmem((nqb, 7, _TQ // 4, D // 2), U32),
                vmem((3, 5, D // 4, D // 2), U32),
                vmem((nqb, _TQ, D), F32),
                vmem((nqb, D // 2, _TQ), U32),
                vmem((2 * D // _LANES, S // 2, _LANES), U32),
                vmem((nqb, D // 2, _TQ), U32),
                vmem((nqb, _H, 8, _TQ), F32),
                vmem((_H, 8, _LANES), F32),
                vmem((_H, nch * _G, _LANES), F32),
                [vmem((_LANES // 2, _TQ), U32)] * nqb,
                [vmem((8, _TQ), F32)] * nqb,
                [vmem((dh, 8, _TQ), F32)] * 2,
                [vmem((dh, nch * _G, _LANES), F32)] * 2,
                vmem((nqb, D, _TQ), F32),
                vmem((nqb, _H, 8, _TQ), F32),
                pltpu.SMEM((1,), jnp.int32),
                pltpu.SemaphoreType.DMA((nqb + 7,)),
                pltpu.SemaphoreType.DMA((nqb + 3,)),
            ],
            compiler_params=pltpu.CompilerParams(vmem_limit_bytes=100 * 1024 * 1024),
            interpret=interpret,
        )(A_x.reshape(S, D), A_wqkv, A_wo, B_w1, B_b1, B_w2)
        return out.reshape(B, S, D)
    return fn


pallas_parallel_sum__mha_block__dense_activation_mish__prompt_kernel = make()
```

```python
import functools
import math

import jax
import jax.numpy as jnp
from jax import lax
import jax.experimental.pallas as pl
import jax.experimental.pallas.tpu as pltpu

_H = 32
_EPS = 1e-5
_LANES = 128
_G = 16
_TQ = 512
_CK = 128
_FB = 384

_LEAD = 2
_VPU_LAG = 8
_VPU_PACE = 2
_STAGE_LAG = 20
_K_PIECES = 4
_K_MARGIN = 2
_Q_EVERY = 2

F32 = jnp.float32
BF16 = jnp.bfloat16
U32 = jnp.uint32


def _pack(a):
    return pltpu.bitcast(a, U32)


def _unpack(a):
    return pltpu.bitcast(a, BF16)


def _vregs(a):
    return a.reshape(a.shape[0] // 8, 8, a.shape[1])


def _widen(a, width):
    return jnp.concatenate([a] * (width // a.shape[-1]), axis=-1)


def _mm(a, b):
    return jnp.dot(a, b, preferred_element_type=F32)


def _recip(a):
    return pltpu.reciprocal(a, approx=True)


def _mish(h):
    e = jnp.exp(jnp.minimum(h, 30.0))
    n = e * (e + 2.0)
    return h * (n * _recip(n + 2.0))


def _quads(a):
    r, c = a.shape[0] // 2, a.shape[1] // 2
    return a[:r, :c], a[:r, c:], a[r:, :c], a[r:, c:]


def _join(c11, c12, c21, c22):
    return jnp.concatenate([jnp.concatenate([c11, c12], axis=1), jnp.concatenate([c21, c22], axis=1)], axis=0)


def _strassen_lhs(a11, a12, a21, a22):
    return [t.astype(BF16) for t in (a21 + a22, a11 + a12, a22, a11, a11 + a22, a21 - a11, a12 - a22)]


def _strassen_rhs(b11, b12, b21, b22):
    f11, f12, f21, f22 = [t.astype(F32) for t in (b11, b12, b21, b22)]
    return [b11, b22] + [t.astype(BF16) for t in (f21 - f11, f12 - f22, f11 + f22, f11 + f12, f21 + f22)]


def _strassen_out(m2, m5, m4, m3, m1, m6, m7):
    return m4 - m5 + m1 + m7, m5 + m3, m2 + m4, m3 - m2 + m1 + m6


def _quad_slices(w_ref, r0, r1, c0, c1):
    r, c = w_ref.shape[0] // 2, w_ref.shape[1] // 2
    return [w_ref[i + r0:i + r1, j + c0:j + c1] for i in (0, r) for j in (0, c)]


def _not_before(true_mask, token):
    def delay(t):
        if token is None:
            return t
        width = t.shape[1]
        return jnp.where(_widen(true_mask, width)[None], _vregs(t), _widen(token, width)[None]).reshape(t.shape)
    return delay


def _kernel(x_hbm, wqkv_hbm, wo_hbm, w1_hbm, b1_hbm, w2_hbm, out_hbm,
            x_v, wqkv_v, wo_v, w1_v, b1_v, w2_v, out_v,
            xa_s, wq_s, qt_s, k_s, vt_s, qn_s, kn_s, kf_s,
            qm_s, shift_s, qb_s, kb_s, ot_s, l_s, carry_s, lo_s, hi_s, zero_s, in_sems, out_sems):
    S, D = x_v.shape
    F = w1_v.shape[1]
    dh = D // _H
    hp = dh // 2
    hpg = _LANES // dh
    nqb = S // _TQ
    nch = S // _CK
    ng = _CK // _G

    zero_s[0] = 0
    always = lax.broadcasted_iota(jnp.int32, (8, _LANES), 0) + zero_s[0] >= 0

    def rows_of(i, n):
        return pl.ds(i * n if isinstance(i, int) else pl.multiple_of(i * n, n), n)

    def clamp(h):
        return jnp.minimum(h, _H - 1)

    def stage_q(h, qb, clear):
        if clear:
            qm_s[qb][rows_of(lax.rem(h + hpg - 1, hpg), hp), :] = jnp.zeros((hp, _TQ), U32)
            qm_s[qb][rows_of(lax.rem(h + hpg // 2 - 1, hpg), hp), :] = jnp.zeros((hp, _TQ), U32)
        qm_s[qb][rows_of(lax.rem(h, hpg), hp), :] = qt_s[qb, rows_of(clamp(h), hp), :]
        norm2 = qn_s[qb, clamp(h)] * _widen(kn_s[clamp(h)], _TQ)
        bound = jnp.exp2(jnp.log(norm2) * (0.5 / math.log(2.0))) * 1.02
        share = (bound * (-1.0 / dh)).astype(BF16).astype(F32)
        shift_s[qb][...] = share * dh
        qm_s[qb][rows_of(lax.rem(h + hpg // 2, hpg), hp), :] = _pack(
            jnp.concatenate([share] * (dh // 8), axis=0).astype(BF16))

    def stage_qb(h, qb, d0, d1, delay):
        r0 = d0 // 8 * 8
        q = delay(_unpack(qt_s[qb, rows_of(clamp(h), hp), :]).astype(F32)[r0:r0 + 8])
        for d in range(d0, d1):
            qb_s[qb % 2][d] = jnp.broadcast_to(q[d - r0:d - r0 + 1], (8, _TQ))

    def stage_kb(h, slot, d, v0, v1, delay):
        k = kf_s[clamp(h), v0 * _G:v1 * _G, :]
        k = jnp.concatenate([delay(k[:8]), k[8:]], axis=0)
        kb_s[slot][d, v0 * _G:v1 * _G, :] = jnp.broadcast_to(k[:, d:d + 1], k.shape)

    todo = []

    def run_todo(n, after=None):
        n = min(n, len(todo))
        for u in range(n):
            r = 0 if after is None else u * (after.shape[0] // 8) // n * 8
            todo.pop(0)(_not_before(always, None if after is None else after[r:r + 8, :_LANES]))

    def weight_pieces(c):
        def piece(r0, delay):
            b = [delay(t.astype(F32)) for t in _quad_slices(wqkv_v.at[c], r0, r0 + _G, 0, D // 2)]
            for n, t in enumerate(_strassen_rhs(*b)[2:]):
                wq_s[c, n, r0 // 2:(r0 + _G) // 2, :] = _pack(t)
        return [functools.partial(piece, r0) for r0 in range(D // 2 - _G, -1, -_G)]

    def layernorm_pieces(i):
        def piece(r0, delay):
            x = [x_v[i * _TQ + t + r0:i * _TQ + t + r0 + _G, :] for t in (0, _TQ // 2)]
            x = delay(jnp.concatenate(x, axis=0).astype(F32))
            xc = x - jnp.mean(x, axis=-1, keepdims=True)
            var = jnp.mean(xc * xc, axis=-1, keepdims=True)
            for n, t in enumerate(_strassen_lhs(*_quads(xc * lax.rsqrt(var + _EPS)))):
                xa_s[i, n, r0 // 2:(r0 + _G) // 2, :] = _pack(t)
        return [functools.partial(piece, r0) for r0 in range(0, _TQ // 2, _G)]

    def project(i, c, rate, wait_at=None, copies=(), weight=None):
        raw = _quad_slices(wqkv_v.at[c], 0, D // 2, 0, D // 2)
        ms = []
        for n in range(7):
            if n == wait_at:
                for cp in copies:
                    cp.wait()
                todo.extend(weight_pieces(weight))
            ms.append(_mm(_unpack(xa_s[i, n]), raw[3 * n] if n < 2 else _unpack(wq_s[c, n - 2])))
            run_todo(rate, ms[-1])
        return _join(*_strassen_out(*ms))

    def head_sum(a):
        return jnp.sum(jnp.sum(a.reshape(_H, dh // 8, 8, a.shape[1]), axis=1), axis=1, keepdims=True)

    def project_k(i, kn, *args):
        k = project(i, 1, *args)
        low = lax.broadcasted_iota(jnp.int32, (_TQ // 2, _LANES), 1) < _LANES // 2
        ones = jnp.full(low.shape, 0x3F803F80, U32)
        for g in range(D // _LANES):
            kg = k[:, g * _LANES:(g + 1) * _LANES]
            kp = _pack(kg.astype(BF16))
            k_s[2 * g, i * _TQ // 2:(i + 1) * _TQ // 2, :] = jnp.where(low, kp, ones)
            k_s[2 * g + 1, i * _TQ // 2:(i + 1) * _TQ // 2, :] = jnp.where(low, ones, kp)
            for j in range(_TQ // _CK):
                kv = kg[(j + 1) * _CK - _G:(j + 1) * _CK]
                v = i * (_TQ // _CK) + j
                for t in range(hpg):
                    kf_s[g * hpg + t, v * _G:(v + 1) * _G, :] = pltpu.roll(kv, _LANES - t * dh, 1) if t else kv
        return jnp.maximum(kn, head_sum(jnp.max((k * k).reshape(_TQ // _LANES, _LANES, D), axis=0).T))

    def project_q(i, *args):
        qt = (project(i, 0, *args) * (dh ** -0.5 * math.log2(math.e))).T
        qt_s[i] = _pack(qt.astype(BF16))
        qn_s[i] = jnp.broadcast_to(head_sum(qt * qt), (_H, 8, _TQ))

    def project_v(i, *args):
        vt_s[i] = _pack(project(i, 2, *args).T.astype(BF16))

    cp_x = [pltpu.make_async_copy(x_hbm.at[i * _TQ:(i + 1) * _TQ], x_v.at[i * _TQ:(i + 1) * _TQ], in_sems.at[i])
            for i in range(nqb)]
    cp_q, cp_k, cp_v = [
        pltpu.make_async_copy(wqkv_hbm.at[:, c * D:(c + 1) * D], wqkv_v.at[c], in_sems.at[nqb + c])
        for c in range(3)]
    cp_rest = [pltpu.make_async_copy(src, dst, in_sems.at[nqb + 3 + n])
               for n, (src, dst) in enumerate([(w1_hbm, w1_v), (b1_hbm, b1_v), (w2_hbm, w2_v), (wo_hbm, wo_v)])]
    for cp in [cp_x[0], cp_k, cp_q, cp_x[1], cp_v] + cp_x[2:] + cp_rest:
        cp.start()
    for qb in range(nqb):
        qm_s[qb][...] = jnp.zeros(qm_s[qb].shape, U32)
    cp_x[0].wait()
    todo += layernorm_pieces(0)
    run_todo(len(todo))
    cp_k.wait()
    todo += weight_pieces(1)
    kn = project_k(0, jnp.zeros((_H, 1, _LANES), F32), 16, 5, [cp_q, cp_x[1]], 0)
    todo += layernorm_pieces(1)
    project_q(0, 3)
    kn = project_k(1, kn, 6, 5, [cp_v] + cp_x[2:], 2)
    project_v(0, 4)
    todo += layernorm_pieces(2)
    project_v(1, 3)
    kn = project_k(2, kn, 0)
    todo += layernorm_pieces(3)
    project_v(2, 3)
    kn = project_k(3, kn, 0)
    kn_s[...] = jnp.broadcast_to(jnp.max(kn, axis=2, keepdims=True), kn_s.shape)
    project_q(1, 0)
    project_q(2, 0)
    project_q(3, 0)
    todo += [functools.partial(stage_kb, 0, 0, d, 0, nch) for d in range(dh)]
    todo += [functools.partial(stage_qb, 0, 0, d, d + 8) for d in range(0, dh, 8)]
    todo += [functools.partial(lambda qb, delay: stage_q(0, qb, False), qb) for qb in range(nqb)]
    project_v(3, 4)
    assert not todo

    order = [j * ng + r for j in range(nch) for r in reversed(range(ng - 1))]
    cuts = [j * (ng - 1) + _LEAD for j in range(nch)] + [len(order)]

    def stream(h0, first, n_qk, n_pv, state):
        zero = zero_s[0]
        l_acc = state
        p_mxu = [carry_s[n + zero] for n in range(ng - 1 + _LEAD)] if first else []
        p_vpu = [carry_s[ng - 1 + _LEAD + zero]] if first else []
        also = lax.broadcasted_iota(jnp.int32, (8, _LANES), 1) + h0 >= 0
        results = []
        staged = []

        def exp_and_sum(s, reset):
            nonlocal l_acc
            p = jnp.exp2(s)
            l_acc = p[:8] if reset else l_acc + p[:8]
            l_acc = l_acc + p[8:]
            return p

        def mxu_scores(item, g0, g1):
            kg = lax.div(clamp(h0 + item // nqb), hpg // 2)
            k = jnp.concatenate([k_s[kg, r * _G // 2:(r + 1) * _G // 2, :] for r in order[g0:g1]], axis=0)
            s = _mm(_unpack(k), _unpack(qm_s[item % nqb][rows_of(zero, _LANES // 2), :]))
            for n in range(g1 - g0):
                results.append(s[(n + 1) * _G - 8:(n + 1) * _G, :_LANES])
                p_mxu.append(exp_and_sum(s[n * _G:(n + 1) * _G], g0 + n == 0))

        def vpu_scores(item, j, slot0):
            qb = item % nqb
            acc = shift_s[qb][rows_of(zero, 8), :][None]
            for d in range(dh):
                k = kb_s[item // nqb % 2][d + zero, j * _G:(j + 1) * _G, :]
                slot = slot0 + d * ng // dh - _VPU_LAG
                if slot >= 0 and d % _VPU_PACE == 0:
                    token = results[slot]
                    while staged:
                        token = jnp.where(always, token, staged.pop())
                    k = _not_before(also, token)(k)
                acc = acc + _widen(_vregs(k), _TQ) * qb_s[qb % 2][d + zero][None]
            p_vpu.append(exp_and_sum(acc.reshape(_G, _TQ), False))

        def next_tile():
            parts = [p_mxu.pop(0) for _ in range(ng - 1)][::-1] + [p_vpu.pop(0)]
            return jnp.concatenate(parts, axis=0).astype(BF16)

        if first == 0:
            mxu_scores(0, 0, _LEAD)
        for t in range(max(n_qk, n_pv)):
            if t < n_qk:
                item, j = divmod(first + t, nch)
                h, qb = h0 + item // nqb, item % nqb
                mxu_scores(item, cuts[j], cuts[j + 1])
                vpu_scores(item, j, t * ng)
                if j == nch - 1:
                    lo_s[...] = jnp.minimum(lo_s[...], l_acc)
                    hi_s[...] = hi_s[...] + l_acc
                    l_s[qb, clamp(h)] = l_acc
                    stage_q(h + 1, qb, True)
                    mxu_scores(item + 1, 0, _LEAD)
                delay = _not_before(also, results[max(len(results) - _STAGE_LAG, 0)])
                if j % _Q_EVERY == _Q_EVERY // 2:
                    d0 = j // _Q_EVERY * _Q_EVERY * dh // nch
                    stage_qb(h + (qb + 1) // nqb, (qb + 1) % nqb, d0, d0 + _Q_EVERY * dh // nch, delay)
                    staged.append(qb_s[(qb + 1) % 2][d0 + zero, :, :_LANES])
                if n_pv:
                    hk, tk = divmod(t, nqb * nch)
                    span, pieces = nqb * nch - first - _K_MARGIN, dh * _K_PIECES
                    for u in range(tk * pieces // span, min((tk + 1) * pieces // span, pieces)):
                        d, v0, v1 = u // _K_PIECES, u % _K_PIECES * nch // _K_PIECES, (u % _K_PIECES + 1) * nch // _K_PIECES
                        stage_kb(h0 + hk + 1, (hk + 1) % 2, d, v0, v1, delay)
                        staged.append(kb_s[(hk + 1) % 2][d + zero, v0 * _G:v0 * _G + 8, :])
            if t < n_pv:
                item, j = divmod(t, nch)
                h = h0 + item // nqb
                blk, off = divmod(j * _CK, _TQ)
                o = _mm(_unpack(vt_s[blk, rows_of(h, hp), off:off + _CK]), next_tile())
                results.append(o[8:, :_LANES])
                o_acc = o if j == 0 else o_acc + o
                if j == nch - 1:
                    ot_s[item % nqb, rows_of(h, dh), :] = o_acc
        for n, p in enumerate(p_mxu + p_vpu):
            carry_s[n] = p
        return l_acc

    lo_s[...] = jnp.ones(lo_s.shape, F32)
    hi_s[...] = jnp.zeros(hi_s.shape, F32)
    state = stream(0, 0, 1, 0, None)
    n = 2 * nqb * nch
    lax.fori_loop(0, _H // 2, lambda i, st: stream(2 * i, 1, n, n, st), state)

    safe = jnp.where((lo_s[...] >= 2.0 ** -64) & (hi_s[...] <= 2.0 ** 40), 1.0, 0.0)

    @pl.when(jnp.min(safe) < 0.5)
    def _():
        def redo(t, carry):
            h, qb = lax.rem(t, _H), lax.div(t, _H)
            qm_s[0][...] = jnp.zeros(qm_s[0].shape, U32)
            qm_s[0][rows_of(lax.rem(h, hpg), hp), :] = qt_s[qb, rows_of(h, hp), :]

            def scores(blk):
                return _mm(_unpack(k_s[lax.div(h, hpg // 2), rows_of(blk, _TQ // 2), :]), _unpack(qm_s[0][...]))

            m = lax.fori_loop(0, nqb, lambda blk, m: jnp.maximum(m, jnp.max(scores(blk), axis=0, keepdims=True)),
                              jnp.full((1, _TQ), -jnp.inf, F32))

            def weigh(blk, sums):
                p = jnp.exp2(scores(blk) - m)
                o = _mm(_unpack(vt_s[blk, rows_of(h, hp), :]), p.astype(BF16))
                return sums[0] + jnp.sum(_vregs(p), axis=0), sums[1] + o

            l, o = lax.fori_loop(0, nqb, weigh, (jnp.zeros((8, _TQ), F32), jnp.zeros((dh, _TQ), F32)))
            l_s[qb, h] = l
            ot_s[qb, rows_of(h, dh), :] = o
            return carry

        lax.fori_loop(0, nqb * _H, redo, 0)

    for cp in cp_rest:
        cp.wait()
    b1 = b1_v[...].astype(F32).reshape(1, F)
    spans = [(f0, min(f0 + _FB, F // 2)) for f0 in range(0, F // 2, _FB)]

    def quadrant(i, u):
        return rows_of(2 * i + u // 2, _TQ // 2), slice(u % 2 * (D // 2), (u % 2 + 1) * (D // 2))

    def out_copy(i, u):
        return pltpu.make_async_copy(out_v.at[quadrant(i, u)], out_hbm.at[quadrant(i, u)], out_sems.at[4 * i + u])

    def finish(i, carry):
        def up(f0, f1):
            ws = _strassen_rhs(*_quad_slices(w1_v, 0, D // 2, f0, f1))
            hs = _strassen_out(*[_mm(_unpack(xa_s[i, n]), ws[n]) for n in range(7)])
            bs = (b1[:, f0:f1], b1[:, F // 2 + f0:F // 2 + f1]) * 2
            return _strassen_lhs(*[_mish(t + b) for t, b in zip(hs, bs)])

        def add_products(acc, lhs, w_ref, r0, r1):
            ms = [_mm(a, w) for a, w in zip(lhs, _strassen_rhs(*_quad_slices(w_ref, r0, r1, 0, D // 2)))]
            return ms if acc is None else [t + m for t, m in zip(acc, ms)]

        act, acc = up(*spans[0]), None
        for u, (f0, f1) in enumerate(spans):
            nxt = up(*spans[u + 1]) if u + 1 < len(spans) else None
            acc = add_products(acc, act, w2_v, f0, f1)
            act = nxt
        o = ot_s[i].reshape(_H, dh, _TQ) * _recip(jnp.sum(l_s[i], axis=1, keepdims=True))
        cs = _strassen_out(*add_products(acc, _strassen_lhs(*_quads(o.reshape(D, _TQ).T)), wo_v, 0, D // 2))
        for u in (1, 2, 3, 0):
            out_v[quadrant(i, u)] = (x_v[quadrant(i, u)].astype(F32) + cs[u]).astype(out_v.dtype)
            out_copy(i, u).start()
        return carry

    lax.fori_loop(0, nqb, finish, 0)
    for i in range(nqb):
        for u in range(4):
            out_copy(i, u).wait()


@jax.jit
def pallas_parallel_sum__mha_block__dense_activation_mish__prompt_kernel(
    A_x: jax.Array,
    A_wqkv: jax.Array,
    A_wo: jax.Array,
    B_x: jax.Array,
    B_w1: jax.Array,
    B_b1: jax.Array,
    B_w2: jax.Array,
):
    del B_x
    B, S, D = A_x.shape
    F = B_w1.shape[1]
    dh, nqb, nch = D // _H, S // _TQ, S // _CK
    assert (B, nqb * _TQ, dh) == (1, S, _G) and nqb == 4 and F % (2 * _LANES) == 0
    hbm = pl.BlockSpec(memory_space=pl.ANY)
    vmem = pltpu.VMEM
    out = pl.pallas_call(
        _kernel,
        in_specs=[hbm] * 6,
        out_specs=hbm,
        out_shape=jax.ShapeDtypeStruct((S, D), A_x.dtype),
        scratch_shapes=[
            vmem((S, D), A_x.dtype),
            vmem((3, D, D), A_wqkv.dtype),
            vmem((D, D), A_wo.dtype),
            vmem((D, F), B_w1.dtype),
            vmem((F,), B_b1.dtype),
            vmem((F, D), B_w2.dtype),
            vmem((S, D), A_x.dtype),
            vmem((nqb, 7, _TQ // 4, D // 2), U32),
            vmem((3, 5, D // 4, D // 2), U32),
            vmem((nqb, D // 2, _TQ), U32),
            vmem((2 * D // _LANES, S // 2, _LANES), U32),
            vmem((nqb, D // 2, _TQ), U32),
            vmem((nqb, _H, 8, _TQ), F32),
            vmem((_H, 8, _LANES), F32),
            vmem((_H, nch * _G, _LANES), F32),
            [vmem((_LANES // 2, _TQ), U32)] * nqb,
            [vmem((8, _TQ), F32)] * nqb,
            [vmem((dh, 8, _TQ), F32)] * 2,
            [vmem((dh, nch * _G, _LANES), F32)] * 2,
            vmem((nqb, D, _TQ), F32),
            vmem((nqb, _H, 8, _TQ), F32),
            vmem((_CK // _G + _LEAD, _G, _TQ), F32),
            vmem((8, _TQ), F32),
            vmem((8, _TQ), F32),
            pltpu.SMEM((1,), jnp.int32),
            pltpu.SemaphoreType.DMA((nqb + 7,)),
            pltpu.SemaphoreType.DMA((4 * nqb,)),
        ],
        compiler_params=pltpu.CompilerParams(vmem_limit_bytes=100 * 1024 * 1024),
    )(A_x.reshape(S, D), A_wqkv, A_wo, B_w1, B_b1, B_w2)
    return out.reshape(B, S, D)
```

```python
import functools
import math

import jax
import jax.numpy as jnp
from jax import lax
import jax.experimental.pallas as pl
import jax.experimental.pallas.tpu as pltpu

_H = 32
_EPS = 1e-5
_LANES = 128
_G = 16
_TQ = 512
_CK = 128
_FB = 384

_LEAD = 2
_VPU_LAG = 8
_VPU_PACE = 2
_STAGE_LAG = 24
_K_PIECES = 4
_K_MARGIN = 2
_Q_EVERY = 2
_HEAD = 5

F32 = jnp.float32
BF16 = jnp.bfloat16
U32 = jnp.uint32


def _pack(a):
    return pltpu.bitcast(a, U32)


def _unpack(a):
    return pltpu.bitcast(a, BF16)


def _vregs(a):
    return a.reshape(a.shape[0] // 8, 8, a.shape[1])


def _widen(a, width):
    return jnp.concatenate([a] * (width // a.shape[-1]), axis=-1)


def _mm(a, b):
    return jnp.dot(a, b, preferred_element_type=F32)


def _recip(a):
    return pltpu.reciprocal(a, approx=True)


def _mish(h):
    e = jnp.exp(jnp.minimum(h, 30.0))
    n = e * (e + 2.0)
    return h * (n * _recip(n + 2.0))


def _quads(a):
    r, c = a.shape[0] // 2, a.shape[1] // 2
    return a[:r, :c], a[:r, c:], a[r:, :c], a[r:, c:]


def _join(c11, c12, c21, c22):
    return jnp.concatenate([jnp.concatenate([c11, c12], axis=1), jnp.concatenate([c21, c22], axis=1)], axis=0)


def _strassen_lhs(a11, a12, a21, a22):
    return [t.astype(BF16) for t in (a21 + a22, a11 + a12, a22, a11, a11 + a22, a21 - a11, a12 - a22)]


def _strassen_rhs(b11, b12, b21, b22):
    f11, f12, f21, f22 = [t.astype(F32) for t in (b11, b12, b21, b22)]
    return [b11, b22] + [t.astype(BF16) for t in (f21 - f11, f12 - f22, f11 + f22, f11 + f12, f21 + f22)]


def _strassen_out(m2, m5, m4, m3, m1, m6, m7):
    return m4 - m5 + m1 + m7, m5 + m3, m2 + m4, m3 - m2 + m1 + m6


def _quad_slices(w_ref, r0, r1, c0, c1):
    r, c = w_ref.shape[0] // 2, w_ref.shape[1] // 2
    return [w_ref[i + r0:i + r1, j + c0:j + c1] for i in (0, r) for j in (0, c)]


def _not_before(true_mask, token):
    def delay(t):
        if token is None:
            return t
        width = t.shape[1]
        return jnp.where(_widen(true_mask, width)[None], _vregs(t), _widen(token, width)[None]).reshape(t.shape)
    return delay


def _kernel(x_hbm, wqkv_hbm, wo_hbm, w1_hbm, b1_hbm, w2_hbm, out_hbm,
            x_v, wqkv_v, wo_v, w1_v, b1_v, w2_v, out_v,
            xa_s, wq_s, qt_s, k_s, vt_s, qn_s, kn_s, kf_s,
            qm_s, shift_s, qb_s, kb_s, ot_s, l_s, carry_s, lo_s, hi_s, zero_s, in_sems, out_sems):
    S, D = x_v.shape
    F = w1_v.shape[1]
    dh = D // _H
    hp = dh // 2
    hpg = _LANES // dh
    nqb = S // _TQ
    nch = S // _CK
    ng = _CK // _G

    zero_s[0] = 0
    always = lax.broadcasted_iota(jnp.int32, (8, _LANES), 0) + zero_s[0] >= 0

    def rows_of(i, n):
        return pl.ds(i * n if isinstance(i, int) else pl.multiple_of(i * n, n), n)

    def clamp(h):
        return jnp.minimum(h, _H - 1)

    def stage_q(h, qb, clear):
        if clear:
            qm_s[qb][rows_of(lax.rem(h + hpg - 1, hpg), hp), :] = jnp.zeros((hp, _TQ), U32)
            qm_s[qb][rows_of(lax.rem(h + hpg // 2 - 1, hpg), hp), :] = jnp.zeros((hp, _TQ), U32)
        qm_s[qb][rows_of(lax.rem(h, hpg), hp), :] = qt_s[qb, rows_of(clamp(h), hp), :]
        norm2 = qn_s[qb, clamp(h)] * _widen(kn_s[clamp(h)], _TQ)
        bound = jnp.exp2(jnp.log(norm2) * (0.5 / math.log(2.0))) * 1.02
        share = (bound * (-1.0 / dh)).astype(BF16).astype(F32)
        shift_s[qb][...] = share * dh
        qm_s[qb][rows_of(lax.rem(h + hpg // 2, hpg), hp), :] = _pack(
            jnp.concatenate([share] * (dh // 8), axis=0).astype(BF16))

    def stage_qb(h, qb, d0, d1, delay):
        r0 = d0 // 8 * 8
        q = delay(_unpack(qt_s[qb, rows_of(clamp(h), hp), :]).astype(F32)[r0:r0 + 8])
        for d in range(d0, d1):
            qb_s[qb % 2][d] = jnp.broadcast_to(q[d - r0:d - r0 + 1], (8, _TQ))

    def stage_kb(h, slot, d, v0, v1, delay):
        k = kf_s[clamp(h), v0 * _G:v1 * _G, :]
        k = jnp.concatenate([delay(k[:8]), k[8:]], axis=0)
        kb_s[slot][d, v0 * _G:v1 * _G, :] = jnp.broadcast_to(k[:, d:d + 1], k.shape)

    todo = []

    def run_todo(n, after=None):
        n = min(n, len(todo))
        for u in range(n):
            r = 0 if after is None else u * (after.shape[0] // 8) // n * 8
            todo.pop(0)(_not_before(always, None if after is None else after[r:r + 8, :_LANES]))

    def weight_pieces(c):
        def piece(r0, delay):
            b = [delay(t.astype(F32)) for t in _quad_slices(wqkv_v.at[c], r0, r0 + _G, 0, D // 2)]
            for n, t in enumerate(_strassen_rhs(*b)[2:]):
                wq_s[c, n, r0 // 2:(r0 + _G) // 2, :] = _pack(t)
        return [functools.partial(piece, r0) for r0 in range(D // 2 - _G, -1, -_G)]

    def layernorm_pieces(i):
        def piece(r0, delay):
            x = [x_v[i * _TQ + t + r0:i * _TQ + t + r0 + _G, :] for t in (0, _TQ // 2)]
            x = delay(jnp.concatenate(x, axis=0).astype(F32))
            xc = x - jnp.mean(x, axis=-1, keepdims=True)
            var = jnp.mean(xc * xc, axis=-1, keepdims=True)
            for n, t in enumerate(_strassen_lhs(*_quads(xc * lax.rsqrt(var + _EPS)))):
                xa_s[i, n, r0 // 2:(r0 + _G) // 2, :] = _pack(t)
        return [functools.partial(piece, r0) for r0 in range(0, _TQ // 2, _G)]

    def project(i, c, rate, wait_at=None, copies=(), weight=None):
        raw = _quad_slices(wqkv_v.at[c], 0, D // 2, 0, D // 2)
        ms = []
        for n in range(7):
            if n == wait_at:
                for cp in copies:
                    cp.wait()
                todo.extend(weight_pieces(weight))
            ms.append(_mm(_unpack(xa_s[i, n]), raw[3 * n] if n < 2 else _unpack(wq_s[c, n - 2])))
            run_todo(rate, ms[-1])
        return _join(*_strassen_out(*ms))

    def head_sum(a):
        return jnp.sum(jnp.sum(a.reshape(_H, dh // 8, 8, a.shape[1]), axis=1), axis=1, keepdims=True)

    def project_k(i, kn, *args):
        k = project(i, 1, *args)
        low = lax.broadcasted_iota(jnp.int32, (_TQ // 2, _LANES), 1) < _LANES // 2
        ones = jnp.full(low.shape, 0x3F803F80, U32)
        for g in range(D // _LANES):
            kg = k[:, g * _LANES:(g + 1) * _LANES]
            kp = _pack(kg.astype(BF16))
            k_s[2 * g, i * _TQ // 2:(i + 1) * _TQ // 2, :] = jnp.where(low, kp, ones)
            k_s[2 * g + 1, i * _TQ // 2:(i + 1) * _TQ // 2, :] = jnp.where(low, ones, kp)
            for j in range(_TQ // _CK):
                kv = kg[(j + 1) * _CK - _G:(j + 1) * _CK]
                v = i * (_TQ // _CK) + j
                for t in range(hpg):
                    kf_s[g * hpg + t, v * _G:(v + 1) * _G, :] = pltpu.roll(kv, _LANES - t * dh, 1) if t else kv
        return jnp.maximum(kn, head_sum(jnp.max((k * k).reshape(_TQ // _LANES, _LANES, D), axis=0).T))

    def project_q(i, *args):
        qt = (project(i, 0, *args) * (dh ** -0.5 * math.log2(math.e))).T
        qt_s[i] = _pack(qt.astype(BF16))
        qn_s[i] = jnp.broadcast_to(head_sum(qt * qt), (_H, 8, _TQ))

    def project_v(i, *args):
        vt_s[i] = _pack(project(i, 2, *args).T.astype(BF16))

    cp_x = [pltpu.make_async_copy(x_hbm.at[i * _TQ:(i + 1) * _TQ], x_v.at[i * _TQ:(i + 1) * _TQ], in_sems.at[i])
            for i in range(nqb)]
    cp_q, cp_k, cp_v = [
        pltpu.make_async_copy(wqkv_hbm.at[:, c * D:(c + 1) * D], wqkv_v.at[c], in_sems.at[nqb + c])
        for c in range(3)]
    cp_rest = [pltpu.make_async_copy(src, dst, in_sems.at[nqb + 3 + n])
               for n, (src, dst) in enumerate([(w1_hbm, w1_v), (b1_hbm, b1_v), (w2_hbm, w2_v), (wo_hbm, wo_v)])]
    for cp in [cp_x[0], cp_k, cp_q, cp_x[1], cp_v] + cp_x[2:] + cp_rest:
        cp.start()
    for qb in range(nqb):
        qm_s[qb][...] = jnp.zeros(qm_s[qb].shape, U32)
    cp_x[0].wait()
    todo += layernorm_pieces(0)
    run_todo(len(todo))
    cp_k.wait()
    todo += weight_pieces(1)
    kn = project_k(0, jnp.zeros((_H, 1, _LANES), F32), 16, 5, [cp_q, cp_x[1]], 0)
    todo += layernorm_pieces(1)
    project_q(0, 3)
    kn = project_k(1, kn, 6, 5, [cp_v] + cp_x[2:], 2)
    project_v(0, 4)
    todo += layernorm_pieces(2)
    project_v(1, 3)
    kn = project_k(2, kn, 0)
    todo += layernorm_pieces(3)
    project_v(2, 3)
    kn = project_k(3, kn, 0)
    kn_s[...] = jnp.broadcast_to(jnp.max(kn, axis=2, keepdims=True), kn_s.shape)
    project_q(1, 0)
    project_q(2, 0)
    project_q(3, 0)
    todo += [functools.partial(stage_kb, 0, 0, d, 0, nch) for d in range(dh)]
    todo += [functools.partial(stage_qb, 0, 0, d, d + 8) for d in range(0, dh, 8)]
    todo += [functools.partial(lambda qb, delay: stage_q(0, qb, False), qb) for qb in range(nqb)]
    project_v(3, 4)
    assert not todo

    order = [j * ng + r for j in range(nch) for r in reversed(range(ng - 1))]
    cuts = [j * (ng - 1) + _LEAD for j in range(nch)] + [len(order)]

    def stream(h0, first, n_qk, n_pv, state):
        zero = zero_s[0]
        l_acc = state
        p_mxu = [carry_s[n + zero] for n in range(ng - 1 + _LEAD)] if first else []
        p_vpu = [carry_s[ng - 1 + _LEAD + zero]] if first else []
        also = lax.broadcasted_iota(jnp.int32, (8, _LANES), 1) + h0 >= 0
        results = []
        staged = []

        def exp_and_sum(s, reset):
            nonlocal l_acc
            p = jnp.exp2(s)
            l_acc = p[:8] if reset else l_acc + p[:8]
            l_acc = l_acc + p[8:]
            return p

        def mxu_scores(item, g0, g1, after=None):
            kg = lax.div(clamp(h0 + item // nqb), hpg // 2)
            k = [k_s[kg, r * _G // 2:(r + 1) * _G // 2, :] for r in order[g0:g1]]
            if after is not None:
                k[_HEAD] = jnp.where(always, k[_HEAD], pltpu.bitcast(after, U32))
            k = jnp.concatenate(k, axis=0)
            s = _mm(_unpack(k), _unpack(qm_s[item % nqb][rows_of(zero, _LANES // 2), :]))
            for n in range(g1 - g0):
                results.append(s[(n + 1) * _G - 8:(n + 1) * _G, :_LANES])
                p_mxu.append(exp_and_sum(s[n * _G:(n + 1) * _G], g0 + n == 0))

        def vpu_scores(item, j, slot0):
            qb = item % nqb
            acc = shift_s[qb][rows_of(zero, 8), :][None]
            for d in range(dh):
                k = kb_s[item // nqb % 2][d + zero, j * _G:(j + 1) * _G, :]
                slot = slot0 + d * ng // dh - _VPU_LAG
                if slot >= 0 and d % _VPU_PACE == 0:
                    token = results[slot]
                    while staged:
                        token = jnp.where(always, token, staged.pop())
                    k = _not_before(also, token)(k)
                acc = acc + _widen(_vregs(k), _TQ) * qb_s[qb % 2][d + zero][None]
            p_vpu.append(exp_and_sum(acc.reshape(_G, _TQ), False))

        def next_tile():
            parts = [p_mxu.pop(0) for _ in range(ng - 1)][::-1] + [p_vpu.pop(0)]
            return jnp.concatenate(parts, axis=0).astype(BF16)

        if first == 0:
            mxu_scores(0, 0, _LEAD)
        for t in range(max(n_qk, n_pv)):
            if t < n_qk:
                item, j = divmod(first + t, nch)
                h, qb = h0 + item // nqb, item % nqb
                if first and t == 0:
                    vpu_scores(item, j, 0)
                    mxu_scores(item, cuts[j], cuts[j + 1], p_vpu[-1][8:, -_LANES:])
                else:
                    mxu_scores(item, cuts[j], cuts[j + 1])
                    vpu_scores(item, j, t * ng)
                if j == nch - 1:
                    lo_s[...] = jnp.minimum(lo_s[...], l_acc)
                    hi_s[...] = hi_s[...] + l_acc
                    l_s[qb, clamp(h)] = l_acc
                    stage_q(h + 1, qb, True)
                    mxu_scores(item + 1, 0, _LEAD)
                delay = _not_before(also, results[max(len(results) - _STAGE_LAG, 0)])
                if j % _Q_EVERY == _Q_EVERY // 2:
                    d0 = j // _Q_EVERY * _Q_EVERY * dh // nch
                    stage_qb(h + (qb + 1) // nqb, (qb + 1) % nqb, d0, d0 + _Q_EVERY * dh // nch, delay)
                    staged.append(qb_s[(qb + 1) % 2][d0 + zero, :, :_LANES])
                if n_pv:
                    hk, tk = divmod(t, nqb * nch)
                    span, pieces = nqb * nch - first - _K_MARGIN, dh * _K_PIECES
                    for u in range(tk * pieces // span, min((tk + 1) * pieces // span, pieces)):
                        d, part = divmod(u, _K_PIECES)
                        v0, v1 = part * nch // _K_PIECES, (part + 1) * nch // _K_PIECES
                        stage_kb(h0 + hk + 1, (hk + 1) % 2, d, v0, v1, delay)
                        staged.append(kb_s[(hk + 1) % 2][d + zero, v0 * _G:v0 * _G + 8, :])
            if t < n_pv:
                item, j = divmod(t, nch)
                h = h0 + item // nqb
                blk, off = divmod(j * _CK, _TQ)
                o = _mm(_unpack(vt_s[blk, rows_of(h, hp), off:off + _CK]), next_tile())
                results.append(o[8:, :_LANES])
                ot_s[item % nqb, rows_of(h, dh), :] = o if j == 0 else ot_s[item % nqb + zero, rows_of(h, dh), :] + o
        for n, p in enumerate(p_mxu + p_vpu):
            carry_s[n] = p
        return l_acc

    lo_s[...] = jnp.ones(lo_s.shape, F32)
    hi_s[...] = jnp.zeros(hi_s.shape, F32)
    state = stream(0, 0, 1, 0, None)
    n = 2 * nqb * nch
    lax.fori_loop(0, _H // 2, lambda i, st: stream(2 * i, 1, n, n, st), state)

    safe = jnp.where((lo_s[...] >= 2.0 ** -64) & (hi_s[...] <= 2.0 ** 40), 1.0, 0.0)

    @pl.when(jnp.min(safe) < 0.5)
    def _():
        def redo(t, carry):
            h, qb = lax.rem(t, _H), lax.div(t, _H)
            qm_s[0][...] = jnp.zeros(qm_s[0].shape, U32)
            qm_s[0][rows_of(lax.rem(h, hpg), hp), :] = qt_s[qb, rows_of(h, hp), :]

            def scores(blk):
                return _mm(_unpack(k_s[lax.div(h, hpg // 2), rows_of(blk, _TQ // 2), :]), _unpack(qm_s[0][...]))

            m = lax.fori_loop(0, nqb, lambda blk, m: jnp.maximum(m, jnp.max(scores(blk), axis=0, keepdims=True)),
                              jnp.full((1, _TQ), -jnp.inf, F32))

            def weigh(blk, sums):
                p = jnp.exp2(scores(blk) - m)
                o = _mm(_unpack(vt_s[blk, rows_of(h, hp), :]), p.astype(BF16))
                return sums[0] + jnp.sum(_vregs(p), axis=0), sums[1] + o

            l, o = lax.fori_loop(0, nqb, weigh, (jnp.zeros((8, _TQ), F32), jnp.zeros((dh, _TQ), F32)))
            l_s[qb, h] = l
            ot_s[qb, rows_of(h, dh), :] = o
            return carry

        lax.fori_loop(0, nqb * _H, redo, 0)

    for cp in cp_rest:
        cp.wait()
    b1 = b1_v[...].astype(F32).reshape(1, F)
    spans = [(f0, min(f0 + _FB, F // 2)) for f0 in range(0, F // 2, _FB)]

    def quadrant(i, u):
        return rows_of(2 * i + u // 2, _TQ // 2), slice(u % 2 * (D // 2), (u % 2 + 1) * (D // 2))

    def out_copy(i, u):
        return pltpu.make_async_copy(out_v.at[quadrant(i, u)], out_hbm.at[quadrant(i, u)], out_sems.at[4 * i + u])

    def finish(i, carry):
        def up(f0, f1):
            ws = _strassen_rhs(*_quad_slices(w1_v, 0, D // 2, f0, f1))
            hs = _strassen_out(*[_mm(_unpack(xa_s[i, n]), ws[n]) for n in range(7)])
            bs = (b1[:, f0:f1], b1[:, F // 2 + f0:F // 2 + f1]) * 2
            return _strassen_lhs(*[_mish(t + b) for t, b in zip(hs, bs)])

        def add_products(acc, lhs, w_ref, r0, r1):
            ms = [_mm(a, w) for a, w in zip(lhs, _strassen_rhs(*_quad_slices(w_ref, r0, r1, 0, D // 2)))]
            return ms if acc is None else [t + m for t, m in zip(acc, ms)]

        act, acc = up(*spans[0]), None
        for u, (f0, f1) in enumerate(spans):
            nxt = up(*spans[u + 1]) if u + 1 < len(spans) else None
            acc = add_products(acc, act, w2_v, f0, f1)
            act = nxt
        o = ot_s[i].reshape(_H, dh, _TQ) * _recip(jnp.sum(l_s[i], axis=1, keepdims=True))
        cs = _strassen_out(*add_products(acc, _strassen_lhs(*_quads(o.reshape(D, _TQ).T)), wo_v, 0, D // 2))
        for u in (1, 2, 3, 0):
            out_v[quadrant(i, u)] = (x_v[quadrant(i, u)].astype(F32) + cs[u]).astype(out_v.dtype)
            out_copy(i, u).start()
        return carry

    lax.fori_loop(0, nqb, finish, 0)
    for i in range(nqb):
        for u in range(4):
            out_copy(i, u).wait()


@jax.jit
def pallas_parallel_sum__mha_block__dense_activation_mish__prompt_kernel(
    A_x: jax.Array,
    A_wqkv: jax.Array,
    A_wo: jax.Array,
    B_x: jax.Array,
    B_w1: jax.Array,
    B_b1: jax.Array,
    B_w2: jax.Array,
):
    del B_x
    B, S, D = A_x.shape
    F = B_w1.shape[1]
    dh, nqb, nch = D // _H, S // _TQ, S // _CK
    assert (B, nqb * _TQ, dh) == (1, S, _G) and nqb == 4 and F % (2 * _LANES) == 0
    hbm = pl.BlockSpec(memory_space=pl.ANY)
    vmem = pltpu.VMEM
    out = pl.pallas_call(
        _kernel,
        in_specs=[hbm] * 6,
        out_specs=hbm,
        out_shape=jax.ShapeDtypeStruct((S, D), A_x.dtype),
        scratch_shapes=[
            vmem((S, D), A_x.dtype),
            vmem((3, D, D), A_wqkv.dtype),
            vmem((D, D), A_wo.dtype),
            vmem((D, F), B_w1.dtype),
            vmem((F,), B_b1.dtype),
            vmem((F, D), B_w2.dtype),
            vmem((S, D), A_x.dtype),
            vmem((nqb, 7, _TQ // 4, D // 2), U32),
            vmem((3, 5, D // 4, D // 2), U32),
            vmem((nqb, D // 2, _TQ), U32),
            vmem((2 * D // _LANES, S // 2, _LANES), U32),
            vmem((nqb, D // 2, _TQ), U32),
            vmem((nqb, _H, 8, _TQ), F32),
            vmem((_H, 8, _LANES), F32),
            vmem((_H, nch * _G, _LANES), F32),
            [vmem((_LANES // 2, _TQ), U32)] * nqb,
            [vmem((8, _TQ), F32)] * nqb,
            [vmem((dh, 8, _TQ), F32)] * 2,
            [vmem((dh, nch * _G, _LANES), F32)] * 2,
            vmem((nqb, D, _TQ), F32),
            vmem((nqb, _H, 8, _TQ), F32),
            vmem((_CK // _G + _LEAD, _G, _TQ), F32),
            vmem((8, _TQ), F32),
            vmem((8, _TQ), F32),
            pltpu.SMEM((1,), jnp.int32),
            pltpu.SemaphoreType.DMA((nqb + 7,)),
            pltpu.SemaphoreType.DMA((4 * nqb,)),
        ],
        compiler_params=pltpu.CompilerParams(vmem_limit_bytes=100 * 1024 * 1024),
    )(A_x.reshape(S, D), A_wqkv, A_wo, B_w1, B_b1, B_w2)
    return out.reshape(B, S, D)
```
